```python
import os as _os
_os.environ.setdefault("JAX_PLATFORMS", "cpu")
import jax
import jax.numpy as jnp

def _softmax(x, axis=-1):
    return jax.nn.softmax(x, axis=axis)
def _gelu(x):
    return jax.nn.gelu(x, approximate=True)
def _silu(x):
    return jax.nn.silu(x)
def _sigmoid(x):
    return jax.nn.sigmoid(x)
def _layernorm(x, axis=-1, eps=1e-5):
    m = jnp.mean(x, axis=axis, keepdims=True)
    v = jnp.var(x, axis=axis, keepdims=True)
    return (x - m) / jnp.sqrt(v + eps)
def _scatter_add(tgt, idx, src, axis=0):
    return tgt.at[idx].add(src)
def _segment_sum(src, seg, n):
    return jax.ops.segment_sum(src, seg, n)
class _Rng:
    def __init__(self, key):
        self._k = key
    def _next(self):
        self._k, sub = jax.random.split(self._k)
        return sub
    def normal(self, shape):
        return jax.random.normal(self._next(), shape, dtype=jnp.bfloat16)
    def randint(self, lo, hi, shape):
        return jax.random.randint(self._next(), shape, lo, hi, dtype=jnp.int32)
    def uniform(self, shape, lo=0.0, hi=1.0):
        return jax.random.uniform(self._next(), shape, jnp.bfloat16, lo, hi)
    def permutation(self, n):
        return jax.random.permutation(self._next(), n)


kernel_name = 'sequential_preLN__softmax_full_mha__swiglu_ffn__prompt'

def setup_inputs():
    _rng = _Rng(jax.random.key(int.from_bytes(__import__("os").urandom(4), "little")))
    _w = (lambda a: (lambda t: t.astype(jnp.bfloat16) if jnp.issubdtype(t.dtype, jnp.floating) else t)(jnp.asarray(a)))
    def _A_setup():
        B, S, D = 1, 2048, 512
        return {
            "x": _w((lambda *s: _rng.normal(s) * 0.05)(B, S, D)),
            "wqkv": _w((lambda *s: _rng.normal(s) * 0.05)(D, 3 * D)),
            "wo": _w((lambda *s: _rng.normal(s) * 0.05)(D, D)),
        }
    _A_in = _A_setup()

    def _B_setup():
        B, S, D, F = 1, 2048, 512, 1792
        return {
            "x": _w((lambda *s: _rng.normal(s) * 0.05)(B, S, D)),
            "w_gate": _w((lambda *s: _rng.normal(s) * 0.05)(D, F)),
            "w_up": _w((lambda *s: _rng.normal(s) * 0.05)(D, F)),
            "w_down": _w((lambda *s: _rng.normal(s) * 0.05)(F, D)),
        }
    _B_in = _B_setup()

    return {
        "A_x": _A_in["x"],
        "A_wqkv": _A_in["wqkv"],
        "A_wo": _A_in["wo"],
        "B_x": _B_in["x"],
        "B_w_gate": _B_in["w_gate"],
        "B_w_up": _B_in["w_up"],
        "B_w_down": _B_in["w_down"],
    }

def reference(A_x, A_wqkv, A_wo, B_x, B_w_gate, B_w_up, B_w_down):
    def _A_ref(x, wqkv, wo):
        B, S, D = x.shape
        H = 32; Dh = D // H
        qkv = (lambda x, *d: x.transpose(*d))((x @ wqkv).reshape(B, S, 3, H, Dh), 2, 0, 3, 1, 4)
        q, k, v = qkv[0], qkv[1], qkv[2]
        scale = Dh ** -0.5
        scores = jnp.einsum("bhqd,bhkd->bhqk", q, k) * scale
        p = _softmax(scores, axis=-1)
        o = jnp.einsum("bhqk,bhkd->bhqd", p, v)
        return (lambda x, *d: x.transpose(*d))(o, 0, 2, 1, 3).reshape(B, S, D) @ wo

    def _B_ref(x, w_gate, w_up, w_down):
        g = _silu(x @ w_gate)
        u = x @ w_up
        return (g * u) @ w_down

    x = A_x
    h = x + _A_ref(_layernorm(x, axis=-1), A_wqkv, A_wo)
    h2 = h + _B_ref(_layernorm(h, axis=-1), B_w_gate, B_w_up, B_w_down)
    return h2
```

```python
import functools
import math

import jax
import jax.numpy as jnp
import jax.experimental.pallas as pl
import jax.experimental.pallas.tpu as pltpu

S, D, H, DH, F = 2048, 512, 32, 16, 1792
EPS = 1e-5
TQ = 512
NQT = S // TQ
CK = 128
NC = S // CK
NU = H * NQT
FC = 256
QSCALE = (DH ** -0.5) * math.log2(math.e)

f32 = jnp.float32
bf16 = jnp.bfloat16
u32 = jnp.uint32


def _ln(xf):
    m = jnp.mean(xf, axis=-1, keepdims=True)
    xc = xf - m
    v = jnp.mean(xc * xc, axis=-1, keepdims=True)
    return xc * jax.lax.rsqrt(v + EPS)


def _kernel(x_hbm, wqkv_hbm, wo_hbm, wg_hbm, wu_hbm, wd_hbm, out_hbm,
            x_v, wqkv_v, wo_v, wg_v, wu_v, wd_v, wqvt_v,
            k_v, qt_v, vt_v, ot_v, sa_v, sb_v, ma_v, mb_v, z_v, out_v,
            xsem, wsem, osem):
    def x_copy(t):
        return pltpu.make_async_copy(x_hbm.at[pl.ds(t * TQ, TQ)], x_v.at[pl.ds(t * TQ, TQ)], xsem.at[t])

    w_copies = [
        pltpu.make_async_copy(wqkv_hbm, wqkv_v, wsem.at[0]),
        pltpu.make_async_copy(wo_hbm, wo_v, wsem.at[1]),
        pltpu.make_async_copy(wg_hbm, wg_v, wsem.at[2]),
        pltpu.make_async_copy(wu_hbm, wu_v, wsem.at[3]),
        pltpu.make_async_copy(wd_hbm, wd_v, wsem.at[4]),
    ]
    x_copy(0).start()
    w_copies[0].start()
    for t in range(1, NQT):
        x_copy(t).start()

    z_v[...] = jnp.zeros_like(z_v)

    w_copies[0].wait()
    for c in w_copies[1:]:
        c.start()

    wq = wqkv_v[:, 0:D].astype(f32)
    wqvt_v[0:D, :] = wq.T.astype(bf16)
    wv = wqkv_v[:, 2 * D:3 * D].astype(f32)
    wqvt_v[D:2 * D, :] = wv.T.astype(bf16)

    for t in range(NQT):
        x_copy(t).wait()
        xn = _ln(x_v[t * TQ:(t + 1) * TQ, :].astype(f32)).astype(bf16)
        kt = jnp.dot(xn, wqkv_v[:, D:2 * D], preferred_element_type=f32).astype(bf16)
        for g in range(4):
            k_v[g, t * (TQ // 2):(t + 1) * (TQ // 2), :] = pltpu.bitcast(kt[:, g * 128:(g + 1) * 128], u32)
        qv = jax.lax.dot_general(wqvt_v[...], xn, (((1,), (1,)), ((), ())),
                                 preferred_element_type=f32)
        qt_v[t] = pltpu.bitcast((qv[0:D] * QSCALE).astype(bf16), u32)
        vt_v[:, t * TQ:(t + 1) * TQ] = pltpu.bitcast(qv[D:2 * D].astype(bf16), u32)

    row_grp = jax.lax.broadcasted_iota(jnp.int32, (64, TQ), 0) // 8

    def unit(u):
        return u // NQT, u % NQT

    def masked_q(u):
        h, qt = unit(u)
        g = h // 8
        qg = qt_v[qt, pl.ds(pl.multiple_of(g * 64, 64), 64), :]
        qm = jnp.where(row_grp == (h % 8), qg, jnp.zeros_like(qg))
        return pltpu.bitcast(qm, bf16)

    def stage1_chunk(g, qm, c, s_ref, macc):
        kc = pltpu.bitcast(k_v[g, c * (CK // 2):(c + 1) * (CK // 2), :], bf16)
        s = jnp.dot(kc, qm, preferred_element_type=f32)
        s_ref[c * CK:(c + 1) * CK, :] = s
        mc = jnp.max(s.reshape(CK // 8, 8, TQ), axis=0)
        return mc if macc is None else jnp.maximum(macc, mc)

    def stage2_chunk(h, c, s_ref, m, acc, lacc):
        s = s_ref[c * CK:(c + 1) * CK, :].reshape(CK // 8, 8, TQ)
        p = jnp.exp2(s - m[None])
        lc = jnp.sum(p, axis=0)
        lacc = lc if lacc is None else lacc + lc
        pb = p.reshape(CK, TQ).astype(bf16)
        vc = pltpu.bitcast(vt_v[pl.ds(pl.multiple_of(h * 8, 8), 8), c * CK:(c + 1) * CK], bf16)
        r = jnp.dot(vc, pb, preferred_element_type=f32)
        return (r if acc is None else acc + r), lacc

    def tie(m, deps, z):
        d = None
        for x in deps:
            if x is None:
                continue
            xb = pltpu.bitcast(x, u32)
            d = xb if d is None else (d | xb)
        if d is None:
            return m
        return pltpu.bitcast(pltpu.bitcast(m, u32) | (d & z), f32)

    def fused(u1, s1_ref, m1_ref, u2, s2_ref, m2_ref, off=1, lag=2):
        if u1 is not None:
            qm = masked_q(u1)
            g1 = unit(u1)[0] // 8
        if u2 is not None:
            h2, qt2 = unit(u2)
            m2 = m2_ref[...]
            z = z_v[...]
        macc = None
        acc = None
        lacc = None
        mhist = []
        for c in range(NC + off):
            if c < NC and u1 is not None:
                macc = stage1_chunk(g1, qm, c, s1_ref, macc)
            mhist.append(macc)
            if c >= off and u2 is not None:
                dm = mhist[c - lag] if c - lag >= 0 else None
                mm = tie(m2, [lacc, dm], z)
                acc, lacc = stage2_chunk(h2, c - off, s2_ref, mm, acc, lacc)
        if u1 is not None:
            m1_ref[...] = jnp.broadcast_to(jnp.max(macc, axis=0, keepdims=True), (8, TQ))
        if u2 is not None:
            l = jnp.sum(lacc, axis=0, keepdims=True)
            ot_v[qt2, pl.ds(pl.multiple_of(h2 * DH, DH), DH), :] = acc * (1.0 / l)

    fused(0, sa_v, ma_v, None, None, None)

    def attn_body(i, carry):
        u = 2 * i
        fused(u + 1, sb_v, mb_v, u, sa_v, ma_v)
        fused(u + 2, sa_v, ma_v, u + 1, sb_v, mb_v)
        return carry

    jax.lax.fori_loop(0, NU // 2 - 1, attn_body, 0)
    fused(NU - 1, sb_v, mb_v, NU - 2, sa_v, ma_v)
    fused(None, None, None, NU - 1, sb_v, mb_v)

    for c in w_copies[1:]:
        c.wait()

    def out_copy(t):
        return pltpu.make_async_copy(out_v.at[t % 2], out_hbm.at[pl.ds(t * TQ, TQ)], osem.at[t % 2])

    for t in range(NQT):
        o = ot_v[t].T.astype(bf16)
        attn = jnp.dot(o, wo_v[...], preferred_element_type=f32)
        hres = x_v[t * TQ:(t + 1) * TQ, :].astype(f32) + attn
        hn = _ln(hres).astype(bf16)
        y = hres
        for fc in range(F // FC):
            gate = jnp.dot(hn, wg_v[:, fc * FC:(fc + 1) * FC], preferred_element_type=f32)
            up = jnp.dot(hn, wu_v[:, fc * FC:(fc + 1) * FC], preferred_element_type=f32)
            hg = 0.5 * gate
            a = ((hg + hg * jnp.tanh(hg)) * up).astype(bf16)
            y = y + jnp.dot(a, wd_v[fc * FC:(fc + 1) * FC, :], preferred_element_type=f32)
        if t >= 2:
            out_copy(t - 2).wait()
        out_v[t % 2] = y.astype(bf16)
        out_copy(t).start()
    out_copy(NQT - 2).wait()
    out_copy(NQT - 1).wait()


@jax.jit
def pallas_sequential_preLN__softmax_full_mha__swiglu_ffn__prompt_kernel(
    A_x: jax.Array,
    A_wqkv: jax.Array,
    A_wo: jax.Array,
    B_x: jax.Array,
    B_w_gate: jax.Array,
    B_w_up: jax.Array,
    B_w_down: jax.Array,
):
    del B_x
    x = A_x.reshape(S, D)
    any_spec = pl.BlockSpec(memory_space=pl.ANY)
    out = pl.pallas_call(
        _kernel,
        out_shape=jax.ShapeDtypeStruct((S, D), bf16),
        in_specs=[any_spec] * 6,
        out_specs=any_spec,
        scratch_shapes=[
            pltpu.VMEM((S, D), bf16),
            pltpu.VMEM((D, 3 * D), bf16),
            pltpu.VMEM((D, D), bf16),
            pltpu.VMEM((D, F), bf16),
            pltpu.VMEM((D, F), bf16),
            pltpu.VMEM((F, D), bf16),
            pltpu.VMEM((2 * D, D), bf16),
            pltpu.VMEM((4, S // 2, 128), u32),
            pltpu.VMEM((NQT, D // 2, TQ), u32),
            pltpu.VMEM((D // 2, S), u32),
            pltpu.VMEM((NQT, D, TQ), f32),
            pltpu.VMEM((S, TQ), f32),
            pltpu.VMEM((S, TQ), f32),
            pltpu.VMEM((8, TQ), f32),
            pltpu.VMEM((8, TQ), f32),
            pltpu.VMEM((8, TQ), u32),
            pltpu.VMEM((2, TQ, D), bf16),
            pltpu.SemaphoreType.DMA((NQT,)),
            pltpu.SemaphoreType.DMA((5,)),
            pltpu.SemaphoreType.DMA((2,)),
        ],
        compiler_params=pltpu.CompilerParams(vmem_limit_bytes=100 * 1024 * 1024),
    )(x, A_wqkv, A_wo, B_w_gate, B_w_up, B_w_down)
    return out.reshape(1, S, D)
```

```python
import functools
import math

import jax
import jax.numpy as jnp
import jax.experimental.pallas as pl
import jax.experimental.pallas.tpu as pltpu

S, D, H, DH, F = 2048, 512, 32, 16, 1792
EPS = 1e-5
TQ = 512
NQT = S // TQ
CK = 128
NC = S // CK
NU = H * NQT
FC = 256
NH = 2
OFF = 2
AD = 12
AE = 4
L_LO = 2.0 ** -30
L_HI = 2.0 ** 60
F_MAX = 3.0e38
QSCALE = (DH ** -0.5) * math.log2(math.e)

f32 = jnp.float32
bf16 = jnp.bfloat16
u32 = jnp.uint32


def _ln(xf):
    m = jnp.mean(xf, axis=-1, keepdims=True)
    xc = xf - m
    v = jnp.mean(xc * xc, axis=-1, keepdims=True)
    return xc * jax.lax.rsqrt(v + EPS)


def _kernel(x_hbm, wqkv_hbm, wo_hbm, wg_hbm, wu_hbm, wd_hbm, out_hbm,
            x_v, wqkv_v, wo_v, wg_v, wu_v, wd_v, wqvt_v,
            k_v, qt_v, vt_v, ot_v, bad_v, z_v, out_v,
            xsem, wsem, osem):
    def x_copy(t):
        return pltpu.make_async_copy(x_hbm.at[pl.ds(t * TQ, TQ)], x_v.at[pl.ds(t * TQ, TQ)], xsem.at[t])

    w_copies = [
        pltpu.make_async_copy(wqkv_hbm, wqkv_v, wsem.at[0]),
        pltpu.make_async_copy(wo_hbm, wo_v, wsem.at[1]),
        pltpu.make_async_copy(wg_hbm, wg_v, wsem.at[2]),
        pltpu.make_async_copy(wu_hbm, wu_v, wsem.at[3]),
        pltpu.make_async_copy(wd_hbm, wd_v, wsem.at[4]),
    ]
    x_copy(0).start()
    w_copies[0].start()
    for t in range(1, NQT):
        x_copy(t).start()

    z_v[...] = jnp.zeros_like(z_v)
    bad_v[...] = jnp.zeros_like(bad_v)

    w_copies[0].wait()
    for c in w_copies[1:]:
        c.start()

    wq = wqkv_v[:, 0:D].astype(f32)
    wqvt_v[0:D, :] = wq.T.astype(bf16)
    wv = wqkv_v[:, 2 * D:3 * D].astype(f32)
    wqvt_v[D:2 * D, :] = wv.T.astype(bf16)

    def phase_a(t, carry):
        x_copy(t).wait()
        r0 = pl.multiple_of(t * TQ, TQ)
        xn = _ln(x_v[pl.ds(r0, TQ), :].astype(f32)).astype(bf16)
        kt = jnp.dot(xn, wqkv_v[:, D:2 * D], preferred_element_type=f32).astype(bf16)
        for g in range(4):
            k_v[g, pl.ds(pl.multiple_of(t * (TQ // 2), TQ // 2), TQ // 2), :] = pltpu.bitcast(kt[:, g * 128:(g + 1) * 128], u32)
        qv = jax.lax.dot_general(wqvt_v[...], xn, (((1,), (1,)), ((), ())),
                                 preferred_element_type=f32)
        qt_v[t] = pltpu.bitcast((qv[0:D] * QSCALE).astype(bf16), u32)
        vt_v[t] = pltpu.bitcast(qv[D:2 * D].astype(bf16), u32)
        return carry

    jax.lax.fori_loop(0, NQT, phase_a, 0)

    row_grp = jax.lax.broadcasted_iota(jnp.int32, (64, TQ), 0) // 8

    def masked_q(h, qt):
        g = h // 8
        qg = qt_v[qt, pl.ds(pl.multiple_of(g * 64, 64), 64), :]
        qm = jnp.where(row_grp == (h % 8), qg, jnp.zeros_like(qg))
        return pltpu.bitcast(qm, bf16)

    def v_chunk(h, c):
        c0 = (c * CK) % TQ
        return vt_v[(c * CK) // TQ, pl.ds(pl.multiple_of(h * 8, 8), 8), c0:c0 + CK]

    def fold(x):
        xb = pltpu.bitcast(x, u32)
        return xb[:, 0:128] | xb[:, 128:256] | xb[:, 256:384] | xb[:, 384:512]

    G = CK // 16

    def stream(h0):
        z = z_v[...]
        n_total = NH * NQT * NC
        deps = {}
        pend = []
        bad = None
        for n in range(n_total + OFF):
            if n < n_total:
                u, c = n // NC, n % NC
                h, qt = h0 + u // NQT, u % NQT
                if c == 0:
                    qm = masked_q(h, qt)
                    lm = None
                g = h // 8
                rows = []
                for gg in range(G):
                    r0 = c * (CK // 2) + gg * 8
                    kv = k_v[g, r0:r0 + 8, :]
                    dep = deps.pop(n * (G + 1) + gg, None)
                    if dep is not None:
                        kv = kv | (dep & z)
                    rows.append(kv)
                kc = pltpu.bitcast(jnp.concatenate(rows, axis=0), bf16)
                s = jnp.dot(kc, qm, preferred_element_type=f32).reshape(2 * G, 8, TQ)
                p = jnp.exp2(s)
                for gg in range(G):
                    t = p[2 * gg] + p[2 * gg + 1]
                    lm = t if lm is None else lm + t
                    if (G - 1 - gg) % AE == 0:
                        sl = n * (G + 1) + gg + AD
                        if sl % (G + 1) == G:
                            sl += 1
                        deps[sl] = fold(lm)
                pend.append((p, lm))
            m = n - OFF
            if m >= 0:
                u, c = m // NC, m % NC
                h, qt = h0 + u // NQT, u % NQT
                p, lm_m = pend[m]
                pend[m] = None
                pb = p.reshape(CK, TQ).astype(bf16)
                r = jnp.dot(pltpu.bitcast(v_chunk(h, c), bf16), pb, preferred_element_type=f32)
                acc = r if c == 0 else acc + r
                if c == NC - 1:
                    l = jnp.sum(lm_m, axis=0, keepdims=True)
                    o = acc * (1.0 / l)
                    ot_v[qt, pl.ds(pl.multiple_of(h * DH, DH), DH), :] = o
                    ok_l = jnp.logical_and(l >= L_LO, l <= L_HI)
                    ok_o = jnp.abs(o) <= F_MAX
                    b = (jnp.where(ok_o[0:8], 0.0, 1.0) + jnp.where(ok_o[8:16], 0.0, 1.0)
                         + jnp.where(ok_l, 0.0, 1.0))
                    bad = b if bad is None else bad + b
        bad_v[...] = bad_v[...] + bad

    def attn_body(i, carry):
        stream(NH * i)
        return carry

    jax.lax.fori_loop(0, H // NH, attn_body, 0)

    @pl.when(jnp.max(bad_v[...]) > 0.0)
    def _():
        def safe_unit(u, carry):
            h, qt = u // NQT, u % NQT
            qm = masked_q(h, qt)
            kg = pltpu.bitcast(k_v[h // 8], bf16)
            s = jnp.dot(kg, qm, preferred_element_type=f32)
            p = jnp.exp2(s - jnp.max(s, axis=0, keepdims=True))
            l = jnp.sum(p, axis=0, keepdims=True)
            pb = p.astype(bf16)
            acc = None
            for t in range(NQT):
                vv = pltpu.bitcast(vt_v[t, pl.ds(pl.multiple_of(h * 8, 8), 8), :], bf16)
                r = jnp.dot(vv, pb[t * TQ:(t + 1) * TQ], preferred_element_type=f32)
                acc = r if acc is None else acc + r
            ot_v[qt, pl.ds(pl.multiple_of(h * DH, DH), DH), :] = acc / l
            return carry

        jax.lax.fori_loop(0, NU, safe_unit, 0)

    for c in w_copies[1:]:
        c.wait()

    def out_copy(t):
        return pltpu.make_async_copy(out_v.at[t % 2], out_hbm.at[pl.ds(t * TQ, TQ)], osem.at[t % 2])

    def phase_c(t, carry):
        r0 = pl.multiple_of(t * TQ, TQ)
        o = ot_v[t].T.astype(bf16)
        attn = jnp.dot(o, wo_v[...], preferred_element_type=f32)
        hres = x_v[pl.ds(r0, TQ), :].astype(f32) + attn
        hn = _ln(hres).astype(bf16)
        y = hres
        for fc in range(F // FC):
            gate = jnp.dot(hn, wg_v[:, fc * FC:(fc + 1) * FC], preferred_element_type=f32)
            up = jnp.dot(hn, wu_v[:, fc * FC:(fc + 1) * FC], preferred_element_type=f32)
            hg = 0.5 * gate
            a = ((hg + hg * jnp.tanh(hg)) * up).astype(bf16)
            y = y + jnp.dot(a, wd_v[fc * FC:(fc + 1) * FC, :], preferred_element_type=f32)

        @pl.when(t >= 2)
        def _():
            out_copy(t - 2).wait()

        out_v[t % 2] = y.astype(bf16)
        out_copy(t).start()
        return carry

    jax.lax.fori_loop(0, NQT, phase_c, 0)
    out_copy(NQT - 2).wait()
    out_copy(NQT - 1).wait()


@jax.jit
def pallas_sequential_preLN__softmax_full_mha__swiglu_ffn__prompt_kernel(
    A_x: jax.Array,
    A_wqkv: jax.Array,
    A_wo: jax.Array,
    B_x: jax.Array,
    B_w_gate: jax.Array,
    B_w_up: jax.Array,
    B_w_down: jax.Array,
):
    del B_x
    x = A_x.reshape(S, D)
    any_spec = pl.BlockSpec(memory_space=pl.ANY)
    out = pl.pallas_call(
        _kernel,
        out_shape=jax.ShapeDtypeStruct((S, D), bf16),
        in_specs=[any_spec] * 6,
        out_specs=any_spec,
        scratch_shapes=[
            pltpu.VMEM((S, D), bf16),
            pltpu.VMEM((D, 3 * D), bf16),
            pltpu.VMEM((D, D), bf16),
            pltpu.VMEM((D, F), bf16),
            pltpu.VMEM((D, F), bf16),
            pltpu.VMEM((F, D), bf16),
            pltpu.VMEM((2 * D, D), bf16),
            pltpu.VMEM((4, S // 2, 128), u32),
            pltpu.VMEM((NQT, D // 2, TQ), u32),
            pltpu.VMEM((NQT, D // 2, TQ), u32),
            pltpu.VMEM((NQT, D, TQ), f32),
            pltpu.VMEM((8, TQ), f32),
            pltpu.VMEM((8, 128), u32),
            pltpu.VMEM((2, TQ, D), bf16),
            pltpu.SemaphoreType.DMA((NQT,)),
            pltpu.SemaphoreType.DMA((5,)),
            pltpu.SemaphoreType.DMA((2,)),
        ],
        compiler_params=pltpu.CompilerParams(vmem_limit_bytes=100 * 1024 * 1024),
    )(x, A_wqkv, A_wo, B_w_gate, B_w_up, B_w_down)
    return out.reshape(1, S, D)
```

```python
import functools
import math

import jax
import jax.numpy as jnp
import jax.experimental.pallas as pl
import jax.experimental.pallas.tpu as pltpu

S, D, H, DH, F = 2048, 512, 32, 16, 1792
EPS = 1e-5
TQ = 512
NQT = S // TQ
CK = 128
NC = S // CK
NU = H * NQT
FC = 256
NH = 2
OFF = 2
AD = 12
AE = 4
NSUB = 2
KS = 256
OSPLIT = 0
L_LO = 2.0 ** -30
L_HI = 2.0 ** 60
F_MAX = 3.0e38
QSCALE = (DH ** -0.5) * math.log2(math.e)

f32 = jnp.float32
bf16 = jnp.bfloat16
u32 = jnp.uint32


def _ln(xf):
    m = jnp.mean(xf, axis=-1, keepdims=True)
    xc = xf - m
    v = jnp.mean(xc * xc, axis=-1, keepdims=True)
    return xc * jax.lax.rsqrt(v + EPS)


def _kernel(x_hbm, wqkv_hbm, wo_hbm, wg_hbm, wu_hbm, wd_hbm, out_hbm,
            x_v, wqkv_v, wo_v, wg_v, wu_v, wd_v, wqvt_v,
            k_v, qt_v, vt_v, ot_v, bad_v, z_v, out_v,
            xsem, wsem, osem):
    def x_copy(t):
        return pltpu.make_async_copy(x_hbm.at[pl.ds(t * TQ, TQ)], x_v.at[pl.ds(t * TQ, TQ)], xsem.at[t])

    def wpart_copy(j):
        return pltpu.make_async_copy(wqkv_hbm.at[:, pl.ds(j * D, D)], wqkv_v.at[j], wsem.at[j])

    w_copies = [
        pltpu.make_async_copy(wo_hbm, wo_v, wsem.at[3]),
        pltpu.make_async_copy(wg_hbm, wg_v, wsem.at[4]),
        pltpu.make_async_copy(wu_hbm, wu_v, wsem.at[5]),
        pltpu.make_async_copy(wd_hbm, wd_v, wsem.at[6]),
    ]
    x_copy(0).start()
    wpart_copy(1).start()

    z_v[...] = jnp.zeros_like(z_v)
    bad_v[...] = jnp.zeros_like(bad_v)

    def ln1(t):
        return _ln(x_v[t * TQ:(t + 1) * TQ, :].astype(f32)).astype(bf16)

    def proj_k(t, xn, lo=0, hi=TQ):
        kt = jnp.dot(xn[lo:hi], wqkv_v[1], preferred_element_type=f32).astype(bf16)
        r0, r1 = (t * TQ + lo) // 2, (t * TQ + hi) // 2
        for g in range(4):
            k_v[g, r0:r1, :] = pltpu.bitcast(kt[:, g * 128:(g + 1) * 128], u32)

    def proj_qv(t, xn):
        qv = jax.lax.dot_general(wqvt_v[...], xn, (((1,), (1,)), ((), ())),
                                 preferred_element_type=f32)
        qt_v[t] = pltpu.bitcast((qv[0:D] * QSCALE).astype(bf16), u32)
        vt_v[t] = pltpu.bitcast(qv[D:2 * D].astype(bf16), u32)

    x_copy(0).wait()
    x_copy(1).start()
    xn0 = ln1(0)
    wpart_copy(1).wait()
    x_copy(2).start()
    proj_k(0, xn0, 0, KS)
    x_copy(1).wait()
    wpart_copy(0).start()
    wpart_copy(2).start()
    x_copy(3).start()
    xn1 = ln1(1)
    proj_k(0, xn0, KS, TQ)
    x_copy(2).wait()
    xn2 = ln1(2)
    proj_k(1, xn1)
    wpart_copy(0).wait()
    wpart_copy(2).wait()
    x_copy(3).wait()
    wqvt_v[0:D, :] = wqkv_v[0].astype(f32).T.astype(bf16)
    wqvt_v[D:2 * D, :] = wqkv_v[2].astype(f32).T.astype(bf16)
    proj_k(2, xn2)
    xn3 = ln1(3)
    proj_qv(0, xn0)
    proj_k(3, xn3)
    proj_qv(1, xn1)
    proj_qv(2, xn2)
    proj_qv(3, xn3)

    row_grp = jax.lax.broadcasted_iota(jnp.int32, (64, TQ), 0) // 8

    def masked_q(h, qt):
        g = h // 8
        qg = qt_v[qt, pl.ds(pl.multiple_of(g * 64, 64), 64), :]
        qm = jnp.where(row_grp == (h % 8), qg, jnp.zeros_like(qg))
        return pltpu.bitcast(qm, bf16)

    def v_chunk(h, c):
        c0 = (c * CK) % TQ
        return vt_v[(c * CK) // TQ, pl.ds(pl.multiple_of(h * 8, 8), 8), c0:c0 + CK]

    def fold(x):
        xb = pltpu.bitcast(x, u32)
        return xb[:, 0:128] | xb[:, 128:256] | xb[:, 256:384] | xb[:, 384:512]

    G = CK // 16

    def stream(h0):
        z = z_v[...]
        n_total = NH * NQT * NC
        deps = {}
        pend = []
        bad = None
        for n in range(n_total + OFF):
            if n < n_total:
                u, c = n // NC, n % NC
                h, qt = h0 + u // NQT, u % NQT
                if c == 0:
                    qm = masked_q(h, qt)
                    lm = None
                g = h // 8
                rows = []
                for gg in range(G):
                    r0 = c * (CK // 2) + gg * 8
                    kv = k_v[g, r0:r0 + 8, :]
                    dep = deps.pop(n * (G + 1) + gg, None)
                    if dep is not None:
                        kv = kv | (dep & z)
                    rows.append(kv)
                kc = pltpu.bitcast(jnp.concatenate(rows, axis=0), bf16)
                s = jnp.dot(kc, qm, preferred_element_type=f32).reshape(2 * G, 8, TQ)
                p = jnp.exp2(s)
                for gg in range(G):
                    t = p[2 * gg] + p[2 * gg + 1]
                    lm = t if lm is None else lm + t
                    if (G - 1 - gg) % AE == 0:
                        sl = n * (G + 1) + gg + AD
                        if sl % (G + 1) == G:
                            sl += 1
                        deps[sl] = fold(lm)
                pend.append((p, lm))
            m = n - OFF
            if m >= 0:
                u, c = m // NC, m % NC
                h, qt = h0 + u // NQT, u % NQT
                p, lm_m = pend[m]
                pend[m] = None
                pb = p.reshape(CK, TQ).astype(bf16)
                r = jnp.dot(pltpu.bitcast(v_chunk(h, c), bf16), pb, preferred_element_type=f32)
                acc = r if c == 0 else acc + r
                if c == NC - 1:
                    l = jnp.sum(lm_m, axis=0, keepdims=True)
                    o = acc * (1.0 / l)
                    ot_v[qt, pl.ds(pl.multiple_of(h * DH, DH), DH), :] = o
                    ok_l = jnp.logical_and(l >= L_LO, l <= L_HI)
                    ok_o = jnp.abs(o) <= F_MAX
                    b = (jnp.where(ok_o[0:8], 0.0, 1.0) + jnp.where(ok_o[8:16], 0.0, 1.0)
                         + jnp.where(ok_l, 0.0, 1.0))
                    bad = b if bad is None else bad + b
        bad_v[...] = bad_v[...] + bad

    def attn_body(i, carry):
        @pl.when(i == 1)
        def _():
            for c in w_copies:
                c.start()

        stream(NH * i)
        return carry

    jax.lax.fori_loop(0, H // NH, attn_body, 0)

    @pl.when(jnp.max(bad_v[...]) > 0.0)
    def _():
        def safe_unit(u, carry):
            h, qt = u // NQT, u % NQT
            qm = masked_q(h, qt)
            kg = pltpu.bitcast(k_v[h // 8], bf16)
            s = jnp.dot(kg, qm, preferred_element_type=f32)
            p = jnp.exp2(s - jnp.max(s, axis=0, keepdims=True))
            l = jnp.sum(p, axis=0, keepdims=True)
            pb = p.astype(bf16)
            acc = None
            for t in range(NQT):
                vv = pltpu.bitcast(vt_v[t, pl.ds(pl.multiple_of(h * 8, 8), 8), :], bf16)
                r = jnp.dot(vv, pb[t * TQ:(t + 1) * TQ], preferred_element_type=f32)
                acc = r if acc is None else acc + r
            ot_v[qt, pl.ds(pl.multiple_of(h * DH, DH), DH), :] = acc / l
            return carry

        jax.lax.fori_loop(0, NU, safe_unit, 0)

    for c in w_copies:
        c.wait()

    HR = TQ // NSUB

    def out_copy(t, a):
        return pltpu.make_async_copy(out_v.at[t % 2, pl.ds(a * HR, HR)],
                                     out_hbm.at[pl.ds(t * TQ + a * HR, HR)], osem.at[(t % 2) * NSUB + a])

    def phase_c(t, carry):
        r0 = pl.multiple_of(t * TQ, TQ)

        @pl.when(t >= 2)
        def _():
            for a in range(NSUB):
                out_copy(t - 2, a).wait()

        hres = []
        for a in range(NSUB):
            o = ot_v[t, :, a * HR:(a + 1) * HR].T.astype(bf16)
            attn = jnp.dot(o, wo_v[...], preferred_element_type=f32)
            hres.append(x_v[pl.ds(r0 + a * HR, HR), :].astype(f32) + attn)
        ys = []
        for a in range(NSUB):
            hn = _ln(hres[a]).astype(bf16)
            y = hres[a]
            for fc in range(F // FC):
                gate = jnp.dot(hn, wg_v[:, fc * FC:(fc + 1) * FC], preferred_element_type=f32)
                up = jnp.dot(hn, wu_v[:, fc * FC:(fc + 1) * FC], preferred_element_type=f32)
                hg = 0.5 * gate
                act = ((hg + hg * jnp.tanh(hg)) * up).astype(bf16)
                y = y + jnp.dot(act, wd_v[fc * FC:(fc + 1) * FC, :], preferred_element_type=f32)
            if OSPLIT:
                out_v[t % 2, a * HR:(a + 1) * HR, :] = y.astype(bf16)
                out_copy(t, a).start()
            else:
                ys.append(y.astype(bf16))
        if not OSPLIT:
            for a in range(NSUB):
                out_v[t % 2, a * HR:(a + 1) * HR, :] = ys[a]
                out_copy(t, a).start()
        return carry

    jax.lax.fori_loop(0, NQT, phase_c, 0)
    for t in range(NQT - 2, NQT):
        for a in range(NSUB):
            out_copy(t, a).wait()


@jax.jit
def pallas_sequential_preLN__softmax_full_mha__swiglu_ffn__prompt_kernel(
    A_x: jax.Array,
    A_wqkv: jax.Array,
    A_wo: jax.Array,
    B_x: jax.Array,
    B_w_gate: jax.Array,
    B_w_up: jax.Array,
    B_w_down: jax.Array,
):
    del B_x
    x = A_x.reshape(S, D)
    any_spec = pl.BlockSpec(memory_space=pl.ANY)
    out = pl.pallas_call(
        _kernel,
        out_shape=jax.ShapeDtypeStruct((S, D), bf16),
        in_specs=[any_spec] * 6,
        out_specs=any_spec,
        scratch_shapes=[
            pltpu.VMEM((S, D), bf16),
            pltpu.VMEM((3, D, D), bf16),
            pltpu.VMEM((D, D), bf16),
            pltpu.VMEM((D, F), bf16),
            pltpu.VMEM((D, F), bf16),
            pltpu.VMEM((F, D), bf16),
            pltpu.VMEM((2 * D, D), bf16),
            pltpu.VMEM((4, S // 2, 128), u32),
            pltpu.VMEM((NQT, D // 2, TQ), u32),
            pltpu.VMEM((NQT, D // 2, TQ), u32),
            pltpu.VMEM((NQT, D, TQ), f32),
            pltpu.VMEM((8, TQ), f32),
            pltpu.VMEM((8, 128), u32),
            pltpu.VMEM((2, TQ, D), bf16),
            pltpu.SemaphoreType.DMA((NQT,)),
            pltpu.SemaphoreType.DMA((7,)),
            pltpu.SemaphoreType.DMA((2 * NSUB,)),
        ],
        compiler_params=pltpu.CompilerParams(vmem_limit_bytes=100 * 1024 * 1024),
    )(x, A_wqkv, A_wo, B_w_gate, B_w_up, B_w_down)
    return out.reshape(1, S, D)
```

```python
import functools
import math

import jax
import jax.numpy as jnp
import jax.experimental.pallas as pl
import jax.experimental.pallas.tpu as pltpu

S, D, H, DH, F = 2048, 512, 32, 16, 1792
EPS = 1e-5
TQ = 512
NQT = S // TQ
CK = 128
NC = S // CK
NU = H * NQT
FC = 256
NH = 2
OFF = 2
AD = 12
AE = 8
NSUB = 2
KS = 256
OSPLIT = 0
VCH = list(range(1, 16, 2))
GL = 1
NG = 4
QC = 3
QN = 8
QVU = 2
L_LO = 2.0 ** -30
L_HI = 2.0 ** 60
F_MAX = 3.0e38
QSCALE = (DH ** -0.5) * math.log2(math.e)

f32 = jnp.float32
bf16 = jnp.bfloat16
u32 = jnp.uint32


def _ln(xf):
    m = jnp.mean(xf, axis=-1, keepdims=True)
    xc = xf - m
    v = jnp.mean(xc * xc, axis=-1, keepdims=True)
    return xc * jax.lax.rsqrt(v + EPS)


def _kernel(x_hbm, wqkv_hbm, wo_hbm, wg_hbm, wu_hbm, wd_hbm, out_hbm,
            x_v, wqkv_v, wo_v, wg_v, wu_v, wd_v, wqvt_v,
            k_v, qt_v, vt_v, ot_v, bad_v, z_v, out_v, ks_v, qb0_v, qb1_v, xn_v,
            xsem, wsem, osem):
    def x_copy(t):
        return pltpu.make_async_copy(x_hbm.at[pl.ds(t * TQ, TQ)], x_v.at[pl.ds(t * TQ, TQ)], xsem.at[t])

    def wpart_copy(j):
        return pltpu.make_async_copy(wqkv_hbm.at[:, pl.ds(j * D, D)], wqkv_v.at[j], wsem.at[j])

    w_copies = [
        pltpu.make_async_copy(wo_hbm, wo_v, wsem.at[3]),
        pltpu.make_async_copy(wg_hbm, wg_v, wsem.at[4]),
        pltpu.make_async_copy(wu_hbm, wu_v, wsem.at[5]),
        pltpu.make_async_copy(wd_hbm, wd_v, wsem.at[6]),
    ]
    x_copy(0).start()
    wpart_copy(1).start()

    z_v[...] = jnp.zeros_like(z_v)
    bad_v[...] = jnp.zeros_like(bad_v)

    def ln1(t):
        xn = _ln(x_v[t * TQ:(t + 1) * TQ, :].astype(f32)).astype(bf16)
        xn_v[t] = pltpu.bitcast(xn, u32)
        return xn

    def proj_k(t, xn, lo=0, hi=TQ):
        kt = jnp.dot(xn[lo:hi], wqkv_v[1], preferred_element_type=f32).astype(bf16)
        r0, r1 = (t * TQ + lo) // 2, (t * TQ + hi) // 2
        for g in range(4):
            k_v[g, r0:r1, :] = pltpu.bitcast(kt[:, g * 128:(g + 1) * 128], u32)
        for ci, c in enumerate(VCH):
            k0 = c * CK - (t * TQ + lo)
            if 0 <= k0 < hi - lo:
                kf = kt[k0:k0 + 16].astype(f32)
                for g in range(4):
                    ks_v[g, ci * 16:(ci + 1) * 16, :] = kf[:, g * 128:(g + 1) * 128]

    def proj_qv(t, xn):
        qv = jax.lax.dot_general(wqvt_v[...], xn, (((1,), (1,)), ((), ())),
                                 preferred_element_type=f32)
        qt_v[t] = pltpu.bitcast((qv[0:D] * QSCALE).astype(bf16), u32)
        vt_v[t] = pltpu.bitcast(qv[D:2 * D].astype(bf16), u32)

    x_copy(0).wait()
    x_copy(1).start()
    xn0 = ln1(0)
    wpart_copy(1).wait()
    x_copy(2).start()
    proj_k(0, xn0, 0, KS)
    x_copy(1).wait()
    wpart_copy(0).start()
    wpart_copy(2).start()
    x_copy(3).start()
    xn1 = ln1(1)
    proj_k(0, xn0, KS, TQ)
    x_copy(2).wait()
    xn2 = ln1(2)
    proj_k(1, xn1)
    wpart_copy(0).wait()
    wpart_copy(2).wait()
    x_copy(3).wait()
    wqvt_v[0:D, :] = wqkv_v[0].astype(f32).T.astype(bf16)
    wqvt_v[D:2 * D, :] = wqkv_v[2].astype(f32).T.astype(bf16)
    proj_k(2, xn2)
    xn3 = ln1(3)
    proj_k(3, xn3)

    def qv_body(t, carry):
        for tt in range(QVU):
            proj_qv(t * QVU + tt, pltpu.bitcast(xn_v[t * QVU + tt], bf16))
        return carry

    jax.lax.fori_loop(0, NQT // QVU, qv_body, 0)

    row_grp = jax.lax.broadcasted_iota(jnp.int32, (64, TQ), 0) // 8

    def q_rows(g, j, qt):
        return qt_v[qt, pl.ds(pl.multiple_of(g * 64 + j * 8, 8), 8), :]

    def masked_q(g, j, qt):
        qh = q_rows(g, j, qt)
        qm = jnp.where(row_grp == j, jnp.concatenate([qh] * 8, axis=0), jnp.zeros((64, TQ), u32))
        return pltpu.bitcast(qm, bf16)

    def v_chunk(h, c):
        c0 = (c * CK) % TQ
        return vt_v[(c * CK) // TQ, pl.ds(pl.multiple_of(h * 8, 8), 8), c0:c0 + CK]

    def fold(x):
        xb = pltpu.bitcast(x, u32)
        return xb[:, 0:128] | xb[:, 128:256] | xb[:, 256:384] | xb[:, 384:512]

    qbs = [qb0_v, qb1_v]

    def qb_make(g, j, qt, dst, ds, gate):
        qu = q_rows(g, j, qt)
        if gate is not None:
            qu = qu | jnp.concatenate([gate] * 4, axis=1)
        for d2 in ds:
            w = jnp.broadcast_to(qu[d2:d2 + 1, :], (8, TQ))
            dst[2 * d2] = pltpu.bitcast(w << 16, f32)
            dst[2 * d2 + 1] = pltpu.bitcast(w & jnp.uint32(0xFFFF0000), f32)

    def vchunk(g, j, qb, ci, gates):
        base = j * 16
        srcs = [ks_v[g, ci * 16 + r * 8:ci * 16 + r * 8 + 8, :] for r in range(2)]
        accs = [None, None]
        for d in range(DH):
            idx = jnp.full((8, 128), base + d, jnp.int32)
            gt = gates[d * len(gates) // DH] if gates else None
            if gt is not None:
                idx = idx | pltpu.bitcast(gt, jnp.int32)
            q = qb[d]
            for r in range(2):
                kb = jnp.take_along_axis(srcs[r], idx, axis=1, mode="promise_in_bounds")
                t = jnp.concatenate([kb] * 4, axis=1) * q
                accs[r] = t if accs[r] is None else accs[r] + t
        return accs

    def stream(i):
        z = z_v[...]
        n_total = 8 * NC
        j = i // 2
        qt0 = 2 * (i % 2)
        Gs = [(7 if (n % NC) in VCH else 8) for n in range(n_total)]
        start = [0]
        for n in range(n_total):
            start.append(start[-1] + Gs[n] + 1)
        qk_slots = set()
        for n in range(n_total):
            for gg in range(Gs[n]):
                qk_slots.add(start[n] + gg)
        deps = {}

        def add_dep(sl, v):
            while sl not in qk_slots and sl < start[-1]:
                sl += 1
            deps.setdefault(sl, []).append(v)

        pend = []
        raw = []
        sv_all = {}
        bad = None
        for n in range(n_total + OFF):
            if n < n_total:
                u, c = n // NC, n % NC
                g, qt = u // 2, qt0 + u % 2
                G = Gs[n]
                nv = CK - 16 * G
                if c == 0:
                    qm = masked_q(g, j, qt)
                    lm = None
                if VCH and QC <= c < QC + QN:
                    un = u + 1
                    if un < 8:
                        nxt = (un // 2, j, qt0 + un % 2)
                    else:
                        nxt = (0, jnp.minimum((i + 1) // 2, 7), 2 - qt0)
                    gate = pltpu.bitcast(raw[n - 2][-1], u32) & z
                    qb_make(*nxt, qbs[un % 2],
                            list(range((c - QC) * 8 // QN, (c - QC + 1) * 8 // QN)), gate)
                m = n + GL - 1
                if m < n_total and (m % NC) in VCH:
                    um = m // NC
                    gsrc = raw[n - 1] if n >= 1 else None
                    gates = [pltpu.bitcast(gsrc[(k + 1) * len(gsrc) // NG - 1], u32) & z
                             for k in range(NG)] if gsrc is not None else None
                    sv_all[m] = vchunk(um // 2, j, qbs[um % 2], VCH.index(m % NC), gates)
                rows = []
                for gg in range(G):
                    r0 = c * (CK // 2) + nv // 2 + gg * 8
                    kv = k_v[g, r0:r0 + 8, :]
                    dl = deps.pop(start[n] + gg, [])
                    if dl:
                        dep = dl[0]
                        for x in dl[1:]:
                            dep = dep | x
                        kv = kv | (dep & z)
                    rows.append(kv)
                kc = pltpu.bitcast(jnp.concatenate(rows, axis=0), bf16)
                s = jnp.dot(kc, qm, preferred_element_type=f32).reshape(2 * G, 8, TQ)
                raw.append([s[2 * gg + 1][:, 0:128] for gg in range(G)])
                p = jnp.exp2(s)
                for gg in range(G):
                    t = p[2 * gg] + p[2 * gg + 1]
                    lm = t if lm is None else lm + t
                    if (G - 1 - gg) % AE == 0:
                        add_dep(start[n] + gg + AD, fold(lm))
                pend.append((p, lm))
            m = n - OFF
            if m >= 0:
                u, c = m // NC, m % NC
                h, qt = (u // 2) * 8 + j, qt0 + u % 2
                if c == 0:
                    lacc = None
                    prev = None
                p, lm_m = pend[m]
                pend[m] = None
                if c in VCH:
                    if m not in sv_all:
                        sv_all[m] = vchunk(u // 2, j, qbs[u % 2], VCH.index(c), None)
                    pv = jnp.exp2(jnp.stack(sv_all.pop(m), axis=0))
                    lc = pv[0] + pv[1]
                    lacc = lc if lacc is None else lacc + lc
                    p = jnp.concatenate([pv, p], axis=0)
                pb = p.reshape(CK, TQ).astype(bf16)
                vu = v_chunk(h, c)
                if prev is not None:
                    vu = vu | (fold(prev) & z)
                prev = lacc if c in VCH else None
                r = jnp.dot(pltpu.bitcast(vu, bf16), pb, preferred_element_type=f32)
                acc = r if c == 0 else acc + r
                if c == NC - 1:
                    lf = lm_m if lacc is None else lm_m + lacc
                    l = jnp.sum(lf, axis=0, keepdims=True)
                    o = acc * (1.0 / l)
                    ot_v[qt, pl.ds(pl.multiple_of(h * DH, DH), DH), :] = o
                    ok_l = jnp.logical_and(l >= L_LO, l <= L_HI)
                    ok_o = jnp.abs(o) <= F_MAX
                    b = (jnp.where(ok_o[0:8], 0.0, 1.0) + jnp.where(ok_o[8:16], 0.0, 1.0)
                         + jnp.where(ok_l, 0.0, 1.0))
                    bad = b if bad is None else bad + b
        bad_v[...] = bad_v[...] + bad

    if VCH:
        qb_make(0, 0, 0, qb0_v, range(8), None)

    def attn_body(i, carry):
        @pl.when(i == 1)
        def _():
            for c in w_copies:
                c.start()

        stream(i)
        return carry

    jax.lax.fori_loop(0, 16, attn_body, 0)

    @pl.when(jnp.max(bad_v[...]) > 0.0)
    def _():
        def safe_unit(u, carry):
            h, qt = u // NQT, u % NQT
            qm = masked_q(h // 8, h % 8, qt)
            kg = pltpu.bitcast(k_v[h // 8], bf16)
            s = jnp.dot(kg, qm, preferred_element_type=f32)
            p = jnp.exp2(s - jnp.max(s, axis=0, keepdims=True))
            l = jnp.sum(p, axis=0, keepdims=True)
            pb = p.astype(bf16)
            acc = None
            for t in range(NQT):
                vv = pltpu.bitcast(vt_v[t, pl.ds(pl.multiple_of(h * 8, 8), 8), :], bf16)
                r = jnp.dot(vv, pb[t * TQ:(t + 1) * TQ], preferred_element_type=f32)
                acc = r if acc is None else acc + r
            ot_v[qt, pl.ds(pl.multiple_of(h * DH, DH), DH), :] = acc / l
            return carry

        jax.lax.fori_loop(0, NU, safe_unit, 0)

    for c in w_copies:
        c.wait()

    HR = TQ // NSUB

    def out_copy(t, a):
        return pltpu.make_async_copy(out_v.at[t % 2, pl.ds(a * HR, HR)],
                                     out_hbm.at[pl.ds(t * TQ + a * HR, HR)], osem.at[(t % 2) * NSUB + a])

    def phase_c(t, carry):
        r0 = pl.multiple_of(t * TQ, TQ)

        @pl.when(t >= 2)
        def _():
            for a in range(NSUB):
                out_copy(t - 2, a).wait()

        hres = []
        for a in range(NSUB):
            o = ot_v[t, :, a * HR:(a + 1) * HR].T.astype(bf16)
            attn = jnp.dot(o, wo_v[...], preferred_element_type=f32)
            hres.append(x_v[pl.ds(r0 + a * HR, HR), :].astype(f32) + attn)
        ys = []
        for a in range(NSUB):
            hn = _ln(hres[a]).astype(bf16)
            y = hres[a]
            for fc in range(F // FC):
                gate = jnp.dot(hn, wg_v[:, fc * FC:(fc + 1) * FC], preferred_element_type=f32)
                up = jnp.dot(hn, wu_v[:, fc * FC:(fc + 1) * FC], preferred_element_type=f32)
                hg = 0.5 * gate
                act = ((hg + hg * jnp.tanh(hg)) * up).astype(bf16)
                y = y + jnp.dot(act, wd_v[fc * FC:(fc + 1) * FC, :], preferred_element_type=f32)
            if OSPLIT:
                out_v[t % 2, a * HR:(a + 1) * HR, :] = y.astype(bf16)
                out_copy(t, a).start()
            else:
                ys.append(y.astype(bf16))
        if not OSPLIT:
            for a in range(NSUB):
                out_v[t % 2, a * HR:(a + 1) * HR, :] = ys[a]
                out_copy(t, a).start()
        return carry

    jax.lax.fori_loop(0, NQT, phase_c, 0)
    for t in range(NQT - 2, NQT):
        for a in range(NSUB):
            out_copy(t, a).wait()


@jax.jit
def pallas_sequential_preLN__softmax_full_mha__swiglu_ffn__prompt_kernel(
    A_x: jax.Array,
    A_wqkv: jax.Array,
    A_wo: jax.Array,
    B_x: jax.Array,
    B_w_gate: jax.Array,
    B_w_up: jax.Array,
    B_w_down: jax.Array,
):
    del B_x
    x = A_x.reshape(S, D)
    any_spec = pl.BlockSpec(memory_space=pl.ANY)
    out = pl.pallas_call(
        _kernel,
        out_shape=jax.ShapeDtypeStruct((S, D), bf16),
        in_specs=[any_spec] * 6,
        out_specs=any_spec,
        scratch_shapes=[
            pltpu.VMEM((S, D), bf16),
            pltpu.VMEM((3, D, D), bf16),
            pltpu.VMEM((D, D), bf16),
            pltpu.VMEM((D, F), bf16),
            pltpu.VMEM((D, F), bf16),
            pltpu.VMEM((F, D), bf16),
            pltpu.VMEM((2 * D, D), bf16),
            pltpu.VMEM((4, S // 2, 128), u32),
            pltpu.VMEM((NQT, D // 2, TQ), u32),
            pltpu.VMEM((NQT, D // 2, TQ), u32),
            pltpu.VMEM((NQT, D, TQ), f32),
            pltpu.VMEM((8, TQ), f32),
            pltpu.VMEM((8, 128), u32),
            pltpu.VMEM((2, TQ, D), bf16),
            pltpu.VMEM((4, 16 * max(len(VCH), 1), 128), f32),
            pltpu.VMEM((DH, 8, TQ), f32),
            pltpu.VMEM((DH, 8, TQ), f32),
            pltpu.VMEM((NQT, TQ // 2, D), u32),
            pltpu.SemaphoreType.DMA((NQT,)),
            pltpu.SemaphoreType.DMA((7,)),
            pltpu.SemaphoreType.DMA((2 * NSUB,)),
        ],
        compiler_params=pltpu.CompilerParams(vmem_limit_bytes=100 * 1024 * 1024),
    )(x, A_wqkv, A_wo, B_w_gate, B_w_up, B_w_down)
    return out.reshape(1, S, D)
```

```python
import math

import jax
import jax.numpy as jnp
import jax.experimental.pallas as pl
import jax.experimental.pallas.tpu as pltpu

S, D, H, DH, F = 2048, 512, 32, 16, 1792
EPS = 1e-5
TQ = 512
NQT = S // TQ
CK = 128
NC = S // CK
NU = H * NQT
FC = 256
OFF = 2
NSUB = 2
KS = 256
QVU = 2
VCH = list(range(1, NC, 2))
AD, ADV, AE, NG, QC, QN = 13, 12, 8, 4, 4, 8
L_LO = 2.0 ** -30
L_HI = 2.0 ** 60
F_MAX = 3.0e38
QSCALE = (DH ** -0.5) * math.log2(math.e)

f32 = jnp.float32
bf16 = jnp.bfloat16
u32 = jnp.uint32


def _ln(xf):
    m = jnp.mean(xf, axis=-1, keepdims=True)
    xc = xf - m
    v = jnp.mean(xc * xc, axis=-1, keepdims=True)
    return xc * jax.lax.rsqrt(v + EPS)


def _kernel(x_hbm, wqkv_hbm, wo_hbm, wg_hbm, wu_hbm, wd_hbm, out_hbm,
            x_v, wqkv_v, wo_v, wg_v, wu_v, wd_v, wqvt_v,
            k_v, qt_v, vt_v, ot_v, bad_v, z_v, out_v, ks_v, qb0_v, qb1_v, xn_v,
            xsem, wsem, osem):
    def x_copy(t):
        return pltpu.make_async_copy(x_hbm.at[pl.ds(t * TQ, TQ)], x_v.at[pl.ds(t * TQ, TQ)], xsem.at[t])

    def wpart_copy(j):
        return pltpu.make_async_copy(wqkv_hbm.at[:, pl.ds(j * D, D)], wqkv_v.at[j], wsem.at[j])

    w_copies = [
        pltpu.make_async_copy(wo_hbm, wo_v, wsem.at[3]),
        pltpu.make_async_copy(wg_hbm, wg_v, wsem.at[4]),
        pltpu.make_async_copy(wu_hbm, wu_v, wsem.at[5]),
        pltpu.make_async_copy(wd_hbm, wd_v, wsem.at[6]),
    ]
    x_copy(0).start()
    wpart_copy(1).start()

    z_v[...] = jnp.zeros_like(z_v)
    bad_v[...] = jnp.zeros_like(bad_v)

    def ln1(t):
        xn = _ln(x_v[t * TQ:(t + 1) * TQ, :].astype(f32)).astype(bf16)
        xn_v[t] = pltpu.bitcast(xn, u32)
        return xn

    def proj_k(t, xn, lo=0, hi=TQ):
        kt = jnp.dot(xn[lo:hi], wqkv_v[1], preferred_element_type=f32).astype(bf16)
        r0, r1 = (t * TQ + lo) // 2, (t * TQ + hi) // 2
        for g in range(4):
            k_v[g, r0:r1, :] = pltpu.bitcast(kt[:, g * 128:(g + 1) * 128], u32)
        for ci, c in enumerate(VCH):
            k0 = c * CK - (t * TQ + lo)
            if 0 <= k0 < hi - lo:
                kf = kt[k0:k0 + 16].astype(f32)
                for g in range(4):
                    ks_v[g, ci * 16:(ci + 1) * 16, :] = kf[:, g * 128:(g + 1) * 128]

    def proj_qv(t, xn):
        qv = jax.lax.dot_general(wqvt_v[...], xn, (((1,), (1,)), ((), ())),
                                 preferred_element_type=f32)
        qt_v[t] = pltpu.bitcast((qv[0:D] * QSCALE).astype(bf16), u32)
        vt_v[t] = pltpu.bitcast(qv[D:2 * D].astype(bf16), u32)

    x_copy(0).wait()
    x_copy(1).start()
    xn0 = ln1(0)
    wpart_copy(1).wait()
    x_copy(2).start()
    proj_k(0, xn0, 0, KS)
    x_copy(1).wait()
    wpart_copy(0).start()
    wpart_copy(2).start()
    x_copy(3).start()
    xn1 = ln1(1)
    proj_k(0, xn0, KS, TQ)
    x_copy(2).wait()
    xn2 = ln1(2)
    proj_k(1, xn1)
    wpart_copy(0).wait()
    wpart_copy(2).wait()
    x_copy(3).wait()
    wqvt_v[0:D, :] = wqkv_v[0].astype(f32).T.astype(bf16)
    wqvt_v[D:2 * D, :] = wqkv_v[2].astype(f32).T.astype(bf16)
    proj_k(2, xn2)
    xn3 = ln1(3)
    proj_k(3, xn3)

    def qv_body(t, carry):
        for tt in range(QVU):
            proj_qv(t * QVU + tt, pltpu.bitcast(xn_v[t * QVU + tt], bf16))
        return carry

    jax.lax.fori_loop(0, NQT // QVU, qv_body, 0)

    row_grp = jax.lax.broadcasted_iota(jnp.int32, (64, TQ), 0) // 8

    def q_rows(g, j, qt):
        return qt_v[qt, pl.ds(pl.multiple_of(g * 64 + j * 8, 8), 8), :]

    def masked_q(g, j, qt):
        qh = q_rows(g, j, qt)
        qm = jnp.where(row_grp == j, jnp.concatenate([qh] * 8, axis=0), jnp.zeros((64, TQ), u32))
        return pltpu.bitcast(qm, bf16)

    def v_chunk(h, c):
        c0 = (c * CK) % TQ
        return vt_v[(c * CK) // TQ, pl.ds(pl.multiple_of(h * 8, 8), 8), c0:c0 + CK]

    def fold(x):
        xb = pltpu.bitcast(x, u32)
        return xb[:, 0:128] | xb[:, 128:256] | xb[:, 256:384] | xb[:, 384:512]

    qbs = [qb0_v, qb1_v]

    def qb_make(g, j, qt, dst, ds, gate):
        qu = q_rows(g, j, qt)
        if gate is not None:
            qu = qu | jnp.concatenate([gate] * 4, axis=1)
        for d2 in ds:
            w = jnp.broadcast_to(qu[d2:d2 + 1, :], (8, TQ))
            dst[2 * d2] = pltpu.bitcast(w << 16, f32)
            dst[2 * d2 + 1] = pltpu.bitcast(w & jnp.uint32(0xFFFF0000), f32)

    def vchunk(g, j, qb, ci, gates):
        base = j * 16
        srcs = [ks_v[g, ci * 16 + r * 8:ci * 16 + r * 8 + 8, :] for r in range(2)]
        accs = [None, None]
        for d in range(DH):
            idx = jnp.full((8, 128), base + d, jnp.int32)
            gt = gates[d * len(gates) // DH] if gates else None
            if gt is not None:
                idx = idx | pltpu.bitcast(gt, jnp.int32)
            q = qb[d]
            for r in range(2):
                kb = jnp.take_along_axis(srcs[r], idx, axis=1, mode="promise_in_bounds")
                t = jnp.concatenate([kb] * 4, axis=1) * q
                accs[r] = t if accs[r] is None else accs[r] + t
        return accs

    def stream(i):
        z = z_v[...]
        n_total = 8 * NC
        j = i // 2
        qt0 = 2 * (i % 2)
        Gs = [(7 if (n % NC) in VCH else 8) for n in range(n_total)]
        start = [0]
        for n in range(n_total):
            start.append(start[-1] + Gs[n] + 1)
        qk_slots = set()
        for n in range(n_total):
            for gg in range(Gs[n]):
                qk_slots.add(start[n] + gg)
        deps = {}

        def add_dep(sl, v):
            while sl not in qk_slots and sl < start[-1]:
                sl += 1
            deps.setdefault(sl, []).append(v)

        pend = []
        raw = []
        sv_all = {}
        bad = None
        for n in range(n_total + OFF):
            if n < n_total:
                u, c = n // NC, n % NC
                g, qt = u // 2, qt0 + u % 2
                G = Gs[n]
                nv = CK - 16 * G
                if c == 0:
                    qm = masked_q(g, j, qt)
                    lm = None
                if QC <= c < QC + QN:
                    un = u + 1
                    if un < 8:
                        nxt = (un // 2, j, qt0 + un % 2)
                    else:
                        nxt = (0, jnp.minimum((i + 1) // 2, 7), 2 - qt0)
                    gate = pltpu.bitcast(raw[n - 2][-1], u32) & z
                    qb_make(*nxt, qbs[un % 2],
                            list(range((c - QC) * 8 // QN, (c - QC + 1) * 8 // QN)), gate)
                if c in VCH:
                    gsrc = raw[n - 1]
                    gates = [pltpu.bitcast(gsrc[(k + 1) * len(gsrc) // NG - 1], u32) & z
                             for k in range(NG)]
                    sv_all[n] = vchunk(g, j, qbs[u % 2], VCH.index(c), gates)
                rows = []
                for gg in range(G):
                    r0 = c * (CK // 2) + nv // 2 + gg * 8
                    kv = k_v[g, r0:r0 + 8, :]
                    dl = deps.pop(start[n] + gg, [])
                    if dl:
                        dep = dl[0]
                        for x in dl[1:]:
                            dep = dep | x
                        kv = kv | (dep & z)
                    rows.append(kv)
                kc = pltpu.bitcast(jnp.concatenate(rows, axis=0), bf16)
                s = jnp.dot(kc, qm, preferred_element_type=f32).reshape(2 * G, 8, TQ)
                raw.append([s[2 * gg + 1][:, 0:128] for gg in range(G)])
                p = jnp.exp2(s)
                for gg in range(G):
                    t = p[2 * gg] + p[2 * gg + 1]
                    lm = t if lm is None else lm + t
                    if (G - 1 - gg) % AE == 0:
                        add_dep(start[n] + gg + (ADV if c in VCH else AD), fold(lm))
                pend.append((p, lm))
            m = n - OFF
            if m >= 0:
                u, c = m // NC, m % NC
                h, qt = (u // 2) * 8 + j, qt0 + u % 2
                if c == 0:
                    lacc = None
                    prev = None
                p, lm_m = pend[m]
                pend[m] = None
                if c in VCH:
                    pv = jnp.exp2(jnp.stack(sv_all.pop(m), axis=0))
                    lc = pv[0] + pv[1]
                    lacc = lc if lacc is None else lacc + lc
                    p = jnp.concatenate([pv, p], axis=0)
                pb = p.reshape(CK, TQ).astype(bf16)
                vu = v_chunk(h, c)
                if prev is not None:
                    vu = vu | (fold(prev) & z)
                prev = lacc if c in VCH else None
                r = jnp.dot(pltpu.bitcast(vu, bf16), pb, preferred_element_type=f32)
                acc = r if c == 0 else acc + r
                if c == NC - 1:
                    lf = lm_m if lacc is None else lm_m + lacc
                    l = jnp.sum(lf, axis=0, keepdims=True)
                    o = acc * (1.0 / l)
                    ot_v[qt, pl.ds(pl.multiple_of(h * DH, DH), DH), :] = o
                    ok_l = jnp.logical_and(l >= L_LO, l <= L_HI)
                    ok_o = jnp.abs(o) <= F_MAX
                    b = (jnp.where(ok_o[0:8], 0.0, 1.0) + jnp.where(ok_o[8:16], 0.0, 1.0)
                         + jnp.where(ok_l, 0.0, 1.0))
                    bad = b if bad is None else bad + b
        bad_v[...] = bad_v[...] + bad

    qb_make(0, 0, 0, qb0_v, range(8), None)

    def attn_body(i, carry):
        @pl.when(i == 1)
        def _():
            for c in w_copies:
                c.start()

        stream(i)
        return carry

    jax.lax.fori_loop(0, 16, attn_body, 0)

    @pl.when(jnp.max(bad_v[...]) > 0.0)
    def _():
        def safe_unit(u, carry):
            h, qt = u // NQT, u % NQT
            qm = masked_q(h // 8, h % 8, qt)
            kg = pltpu.bitcast(k_v[h // 8], bf16)
            s = jnp.dot(kg, qm, preferred_element_type=f32)
            p = jnp.exp2(s - jnp.max(s, axis=0, keepdims=True))
            l = jnp.sum(p, axis=0, keepdims=True)
            pb = p.astype(bf16)
            acc = None
            for t in range(NQT):
                vv = pltpu.bitcast(vt_v[t, pl.ds(pl.multiple_of(h * 8, 8), 8), :], bf16)
                r = jnp.dot(vv, pb[t * TQ:(t + 1) * TQ], preferred_element_type=f32)
                acc = r if acc is None else acc + r
            ot_v[qt, pl.ds(pl.multiple_of(h * DH, DH), DH), :] = acc / l
            return carry

        jax.lax.fori_loop(0, NU, safe_unit, 0)

    for c in w_copies:
        c.wait()

    HR = TQ // NSUB

    def out_copy(t, a):
        return pltpu.make_async_copy(out_v.at[t % 2, pl.ds(a * HR, HR)],
                                     out_hbm.at[pl.ds(t * TQ + a * HR, HR)], osem.at[(t % 2) * NSUB + a])

    def phase_c(t, carry):
        r0 = pl.multiple_of(t * TQ, TQ)

        @pl.when(t >= 2)
        def _():
            for a in range(NSUB):
                out_copy(t - 2, a).wait()

        hres = []
        for a in range(NSUB):
            o = ot_v[t, :, a * HR:(a + 1) * HR].T.astype(bf16)
            attn = jnp.dot(o, wo_v[...], preferred_element_type=f32)
            hres.append(x_v[pl.ds(r0 + a * HR, HR), :].astype(f32) + attn)
        ys = []
        for a in range(NSUB):
            hn = _ln(hres[a]).astype(bf16)
            y = hres[a]
            for fc in range(F // FC):
                gate = jnp.dot(hn, wg_v[:, fc * FC:(fc + 1) * FC], preferred_element_type=f32)
                up = jnp.dot(hn, wu_v[:, fc * FC:(fc + 1) * FC], preferred_element_type=f32)
                hg = 0.5 * gate
                act = ((hg + hg * jnp.tanh(hg)) * up).astype(bf16)
                y = y + jnp.dot(act, wd_v[fc * FC:(fc + 1) * FC, :], preferred_element_type=f32)
            ys.append(y.astype(bf16))
        for a in range(NSUB):
            out_v[t % 2, a * HR:(a + 1) * HR, :] = ys[a]
            out_copy(t, a).start()
        return carry

    jax.lax.fori_loop(0, NQT, phase_c, 0)
    for t in range(NQT - 2, NQT):
        for a in range(NSUB):
            out_copy(t, a).wait()


@jax.jit
def pallas_sequential_preLN__softmax_full_mha__swiglu_ffn__prompt_kernel(
    A_x: jax.Array,
    A_wqkv: jax.Array,
    A_wo: jax.Array,
    B_x: jax.Array,
    B_w_gate: jax.Array,
    B_w_up: jax.Array,
    B_w_down: jax.Array,
):
    del B_x
    x = A_x.reshape(S, D)
    any_spec = pl.BlockSpec(memory_space=pl.ANY)
    out = pl.pallas_call(
        _kernel,
        out_shape=jax.ShapeDtypeStruct((S, D), bf16),
        in_specs=[any_spec] * 6,
        out_specs=any_spec,
        scratch_shapes=[
            pltpu.VMEM((S, D), bf16),
            pltpu.VMEM((3, D, D), bf16),
            pltpu.VMEM((D, D), bf16),
            pltpu.VMEM((D, F), bf16),
            pltpu.VMEM((D, F), bf16),
            pltpu.VMEM((F, D), bf16),
            pltpu.VMEM((2 * D, D), bf16),
            pltpu.VMEM((4, S // 2, 128), u32),
            pltpu.VMEM((NQT, D // 2, TQ), u32),
            pltpu.VMEM((NQT, D // 2, TQ), u32),
            pltpu.VMEM((NQT, D, TQ), f32),
            pltpu.VMEM((8, TQ), f32),
            pltpu.VMEM((8, 128), u32),
            pltpu.VMEM((2, TQ, D), bf16),
            pltpu.VMEM((4, 16 * len(VCH), 128), f32),
            pltpu.VMEM((DH, 8, TQ), f32),
            pltpu.VMEM((DH, 8, TQ), f32),
            pltpu.VMEM((NQT, TQ // 2, D), u32),
            pltpu.SemaphoreType.DMA((NQT,)),
            pltpu.SemaphoreType.DMA((7,)),
            pltpu.SemaphoreType.DMA((2 * NSUB,)),
        ],
        compiler_params=pltpu.CompilerParams(vmem_limit_bytes=100 * 1024 * 1024),
    )(x, A_wqkv, A_wo, B_w_gate, B_w_up, B_w_down)
    return out.reshape(1, S, D)
```

```python
import math

import jax
import jax.numpy as jnp
import jax.experimental.pallas as pl
import jax.experimental.pallas.tpu as pltpu

S, D, H, DH, F = 2048, 512, 32, 16, 1792
EPS = 1e-5
TQ = 512
NQT = S // TQ
CK = 128
NC = S // CK
NU = H * NQT
FC = 256
OFF = 2
NSUB = 2
KS = 256
QVU = 2
VCH = list(range(2, NC))
AD, ADV, AE, NG, QC, QN = 13, 12, 4, 7, 5, 8
L_LO = 2.0 ** -30
L_HI = 2.0 ** 60
F_MAX = 3.0e38
QSCALE = (DH ** -0.5) * math.log2(math.e)

f32 = jnp.float32
bf16 = jnp.bfloat16
u32 = jnp.uint32


def _ln(xf):
    m = jnp.mean(xf, axis=-1, keepdims=True)
    xc = xf - m
    v = jnp.mean(xc * xc, axis=-1, keepdims=True)
    return xc * jax.lax.rsqrt(v + EPS)


def _kernel(x_hbm, wqkv_hbm, wo_hbm, wg_hbm, wu_hbm, wd_hbm, out_hbm,
            x_v, wqkv_v, wo_v, wg_v, wu_v, wd_v, wqvt_v,
            k_v, qt_v, vt_v, ot_v, bad_v, z_v, out_v, ks_v, qb0_v, qb1_v, xn_v,
            xsem, wsem, osem):
    def x_copy(t):
        return pltpu.make_async_copy(x_hbm.at[pl.ds(t * TQ, TQ)], x_v.at[pl.ds(t * TQ, TQ)], xsem.at[t])

    def wpart_copy(j):
        return pltpu.make_async_copy(wqkv_hbm.at[:, pl.ds(j * D, D)], wqkv_v.at[j], wsem.at[j])

    w_copies = [
        pltpu.make_async_copy(wo_hbm, wo_v, wsem.at[3]),
        pltpu.make_async_copy(wg_hbm, wg_v, wsem.at[4]),
        pltpu.make_async_copy(wu_hbm, wu_v, wsem.at[5]),
        pltpu.make_async_copy(wd_hbm, wd_v, wsem.at[6]),
    ]
    x_copy(0).start()
    wpart_copy(1).start()

    z_v[...] = jnp.zeros_like(z_v)
    bad_v[...] = jnp.zeros_like(bad_v)

    def ln1(t):
        xn = _ln(x_v[t * TQ:(t + 1) * TQ, :].astype(f32)).astype(bf16)
        xn_v[t] = pltpu.bitcast(xn, u32)
        return xn

    def proj_k(t, xn, lo=0, hi=TQ):
        kt = jnp.dot(xn[lo:hi], wqkv_v[1], preferred_element_type=f32).astype(bf16)
        r0, r1 = (t * TQ + lo) // 2, (t * TQ + hi) // 2
        for g in range(4):
            k_v[g, r0:r1, :] = pltpu.bitcast(kt[:, g * 128:(g + 1) * 128], u32)
        for ci, c in enumerate(VCH):
            k0 = c * CK - (t * TQ + lo)
            if 0 <= k0 < hi - lo:
                kb = pltpu.bitcast(kt[k0:k0 + 16].astype(f32), u32)
                kw = (kb[0:8] >> 16) | kb[8:16]
                for g in range(4):
                    ks_v[g, ci * 8:(ci + 1) * 8, :] = kw[:, g * 128:(g + 1) * 128]

    def proj_qv(t, xn):
        qv = jax.lax.dot_general(wqvt_v[...], xn, (((1,), (1,)), ((), ())),
                                 preferred_element_type=f32)
        qt_v[t] = pltpu.bitcast((qv[0:D] * QSCALE).astype(bf16), u32)
        vt_v[t] = pltpu.bitcast(qv[D:2 * D].astype(bf16), u32)

    x_copy(0).wait()
    x_copy(1).start()
    xn0 = ln1(0)
    wpart_copy(1).wait()
    x_copy(2).start()
    proj_k(0, xn0, 0, KS)
    x_copy(1).wait()
    wpart_copy(0).start()
    wpart_copy(2).start()
    x_copy(3).start()
    xn1 = ln1(1)
    proj_k(0, xn0, KS, TQ)
    x_copy(2).wait()
    xn2 = ln1(2)
    proj_k(1, xn1)
    wpart_copy(0).wait()
    wpart_copy(2).wait()
    x_copy(3).wait()
    wqvt_v[0:D, :] = wqkv_v[0].astype(f32).T.astype(bf16)
    wqvt_v[D:2 * D, :] = wqkv_v[2].astype(f32).T.astype(bf16)
    proj_k(2, xn2)
    xn3 = ln1(3)
    proj_k(3, xn3)

    def qv_body(t, carry):
        for tt in range(QVU):
            proj_qv(t * QVU + tt, pltpu.bitcast(xn_v[t * QVU + tt], bf16))
        return carry

    jax.lax.fori_loop(0, NQT // QVU, qv_body, 0)

    row_grp = jax.lax.broadcasted_iota(jnp.int32, (64, TQ), 0) // 8

    def q_rows(g, j, qt):
        return qt_v[qt, pl.ds(pl.multiple_of(g * 64 + j * 8, 8), 8), :]

    def masked_q(g, j, qt):
        qh = q_rows(g, j, qt)
        qm = jnp.where(row_grp == j, jnp.concatenate([qh] * 8, axis=0), jnp.zeros((64, TQ), u32))
        return pltpu.bitcast(qm, bf16)

    def v_chunk(h, c):
        c0 = (c * CK) % TQ
        return vt_v[(c * CK) // TQ, pl.ds(pl.multiple_of(h * 8, 8), 8), c0:c0 + CK]

    def fold(x):
        xb = pltpu.bitcast(x, u32)
        return xb[:, 0:128] | xb[:, 128:256] | xb[:, 256:384] | xb[:, 384:512]

    qbs = [qb0_v, qb1_v]

    def qb_make(g, j, qt, dst, ds, gate):
        qu = q_rows(g, j, qt)
        if gate is not None:
            qu = qu | jnp.concatenate([gate] * 4, axis=1)
        for d2 in ds:
            w = jnp.broadcast_to(qu[d2:d2 + 1, :], (8, TQ))
            dst[2 * d2] = pltpu.bitcast(w << 16, f32)
            dst[2 * d2 + 1] = pltpu.bitcast(w & jnp.uint32(0xFFFF0000), f32)

    def vchunk(g, base, qb, ci, gates):
        src = ks_v[g, ci * 8:(ci + 1) * 8, :]
        accs = [None, None]
        gb = None
        for d in range(DH):
            k = d * len(gates) // DH
            if gb is None or k != gb[0]:
                gb = (k, base | pltpu.bitcast(gates[k], jnp.int32))
            idx = gb[1] + d if d else gb[1]
            q = qb[d]
            w = jnp.take_along_axis(src, idx, axis=1, mode="promise_in_bounds")
            kbs = [pltpu.bitcast(w << 16, f32), pltpu.bitcast(w & jnp.uint32(0xFFFF0000), f32)]
            for r in range(2):
                t = jnp.concatenate([kbs[r]] * 4, axis=1) * q
                accs[r] = t if accs[r] is None else accs[r] + t
        return accs

    def stream(i):
        z = z_v[...]
        n_total = 8 * NC
        j = i // 2
        qt0 = 2 * (i % 2)
        base = jnp.full((8, 128), j * DH, jnp.int32)
        Gs = [(7 if (n % NC) in VCH else 8) for n in range(n_total)]
        start = [0]
        for n in range(n_total):
            start.append(start[-1] + Gs[n] + 1)
        qk_slots = set()
        for n in range(n_total):
            for gg in range(Gs[n]):
                qk_slots.add(start[n] + gg)
        deps = {}

        def add_dep(sl, v):
            while sl not in qk_slots and sl < start[-1]:
                sl += 1
            deps.setdefault(sl, []).append(v)

        pend = []
        raw = []
        sv_all = {}
        bad = None
        extra = None
        for n in range(n_total + OFF):
            if n < n_total:
                u, c = n // NC, n % NC
                g, qt = u // 2, qt0 + u % 2
                G = Gs[n]
                nv = CK - 16 * G
                if c == 0:
                    qm = masked_q(g, j, qt)
                    lm = None
                if QC <= c < QC + QN:
                    un = u + 1
                    if un < 8:
                        nxt = (un // 2, j, qt0 + un % 2)
                    else:
                        nxt = (0, jnp.minimum((i + 1) // 2, 7), 2 - qt0)
                    gate = pltpu.bitcast(raw[n - 2][-1], u32) & z
                    qb_make(*nxt, qbs[un % 2],
                            list(range((c - QC) * 8 // QN, (c - QC + 1) * 8 // QN)), gate)
                if c in VCH:
                    gsrc = raw[n - 1]
                    gates = [pltpu.bitcast(gsrc[(k + 1) * len(gsrc) // NG - 1], u32) & z
                             for k in range(NG)]
                    sv_all[n] = vchunk(g, base, qbs[u % 2], VCH.index(c), gates)
                rows = []
                for gg in range(G):
                    r0 = c * (CK // 2) + nv // 2 + gg * 8
                    kv = k_v[g, r0:r0 + 8, :]
                    dl = deps.pop(start[n] + gg, [])
                    if dl:
                        dep = dl[0]
                        for x in dl[1:]:
                            dep = dep | x
                        kv = kv | (dep & z)
                    rows.append(kv)
                kc = pltpu.bitcast(jnp.concatenate(rows, axis=0), bf16)
                s = jnp.dot(kc, qm, preferred_element_type=f32).reshape(2 * G, 8, TQ)
                raw.append([s[2 * gg + 1][:, 0:128] for gg in range(G)])
                p = jnp.exp2(s)
                if extra is not None:
                    lm = lm + extra
                    extra = None
                for gg in range(G):
                    t = p[2 * gg] + p[2 * gg + 1]
                    lm = t if lm is None else lm + t
                    if (G - 1 - gg) % AE == 0:
                        add_dep(start[n] + gg + (ADV if c in VCH else AD), fold(lm))
                pend.append((p, lm))
            m = n - OFF
            if m >= 0:
                u, c = m // NC, m % NC
                h, qt = (u // 2) * 8 + j, qt0 + u % 2
                if c == 0:
                    lacc = None
                    prev = None
                p, lm_m = pend[m]
                pend[m] = None
                if c in VCH:
                    pv = jnp.exp2(jnp.stack(sv_all.pop(m), axis=0))
                    lc = pv[0] + pv[1]
                    if n + 1 < n_total and (n + 1) // NC == u:
                        extra = lc
                    else:
                        lacc = lc if lacc is None else lacc + lc
                    p = jnp.concatenate([pv, p], axis=0)
                pb = p.reshape(CK, TQ).astype(bf16)
                vu = v_chunk(h, c)
                if prev is not None:
                    vu = vu | (fold(prev) & z)
                prev = lacc if (c in VCH and extra is None) else None
                r = jnp.dot(pltpu.bitcast(vu, bf16), pb, preferred_element_type=f32)
                acc = r if c == 0 else acc + r
                if c == NC - 1:
                    lf = lm_m if lacc is None else lm_m + lacc
                    l = jnp.sum(lf, axis=0, keepdims=True)
                    o = acc * (1.0 / l)
                    ot_v[qt, pl.ds(pl.multiple_of(h * DH, DH), DH), :] = o
                    ok_l = jnp.logical_and(l >= L_LO, l <= L_HI)
                    ok_o = jnp.abs(o) <= F_MAX
                    b = (jnp.where(ok_o[0:8], 0.0, 1.0) + jnp.where(ok_o[8:16], 0.0, 1.0)
                         + jnp.where(ok_l, 0.0, 1.0))
                    bad = b if bad is None else bad + b
        bad_v[...] = bad_v[...] + bad

    qb_make(0, 0, 0, qb0_v, range(8), None)

    def attn_body(i, carry):
        @pl.when(i == 1)
        def _():
            for c in w_copies:
                c.start()

        stream(i)
        return carry

    jax.lax.fori_loop(0, 16, attn_body, 0)

    @pl.when(jnp.max(bad_v[...]) > 0.0)
    def _():
        def safe_unit(u, carry):
            h, qt = u // NQT, u % NQT
            qm = masked_q(h // 8, h % 8, qt)
            kg = pltpu.bitcast(k_v[h // 8], bf16)
            s = jnp.dot(kg, qm, preferred_element_type=f32)
            p = jnp.exp2(s - jnp.max(s, axis=0, keepdims=True))
            l = jnp.sum(p, axis=0, keepdims=True)
            pb = p.astype(bf16)
            acc = None
            for t in range(NQT):
                vv = pltpu.bitcast(vt_v[t, pl.ds(pl.multiple_of(h * 8, 8), 8), :], bf16)
                r = jnp.dot(vv, pb[t * TQ:(t + 1) * TQ], preferred_element_type=f32)
                acc = r if acc is None else acc + r
            ot_v[qt, pl.ds(pl.multiple_of(h * DH, DH), DH), :] = acc / l
            return carry

        jax.lax.fori_loop(0, NU, safe_unit, 0)

    for c in w_copies:
        c.wait()

    HR = TQ // NSUB

    def out_copy(t, a):
        return pltpu.make_async_copy(out_v.at[t % 2, pl.ds(a * HR, HR)],
                                     out_hbm.at[pl.ds(t * TQ + a * HR, HR)], osem.at[(t % 2) * NSUB + a])

    def phase_c(t, carry):
        r0 = pl.multiple_of(t * TQ, TQ)

        @pl.when(t >= 2)
        def _():
            for a in range(NSUB):
                out_copy(t - 2, a).wait()

        hres = []
        for a in range(NSUB):
            o = ot_v[t, :, a * HR:(a + 1) * HR].T.astype(bf16)
            attn = jnp.dot(o, wo_v[...], preferred_element_type=f32)
            hres.append(x_v[pl.ds(r0 + a * HR, HR), :].astype(f32) + attn)
        ys = []
        for a in range(NSUB):
            hn = _ln(hres[a]).astype(bf16)
            y = hres[a]
            for fc in range(F // FC):
                gate = jnp.dot(hn, wg_v[:, fc * FC:(fc + 1) * FC], preferred_element_type=f32)
                up = jnp.dot(hn, wu_v[:, fc * FC:(fc + 1) * FC], preferred_element_type=f32)
                hg = 0.5 * gate
                act = ((hg + hg * jnp.tanh(hg)) * up).astype(bf16)
                y = y + jnp.dot(act, wd_v[fc * FC:(fc + 1) * FC, :], preferred_element_type=f32)
            ys.append(y.astype(bf16))
        for a in range(NSUB):
            out_v[t % 2, a * HR:(a + 1) * HR, :] = ys[a]
            out_copy(t, a).start()
        return carry

    jax.lax.fori_loop(0, NQT, phase_c, 0)
    for t in range(NQT - 2, NQT):
        for a in range(NSUB):
            out_copy(t, a).wait()


@jax.jit
def pallas_sequential_preLN__softmax_full_mha__swiglu_ffn__prompt_kernel(
    A_x: jax.Array,
    A_wqkv: jax.Array,
    A_wo: jax.Array,
    B_x: jax.Array,
    B_w_gate: jax.Array,
    B_w_up: jax.Array,
    B_w_down: jax.Array,
):
    del B_x
    x = A_x.reshape(S, D)
    any_spec = pl.BlockSpec(memory_space=pl.ANY)
    out = pl.pallas_call(
        _kernel,
        out_shape=jax.ShapeDtypeStruct((S, D), bf16),
        in_specs=[any_spec] * 6,
        out_specs=any_spec,
        scratch_shapes=[
            pltpu.VMEM((S, D), bf16),
            pltpu.VMEM((3, D, D), bf16),
            pltpu.VMEM((D, D), bf16),
            pltpu.VMEM((D, F), bf16),
            pltpu.VMEM((D, F), bf16),
            pltpu.VMEM((F, D), bf16),
            pltpu.VMEM((2 * D, D), bf16),
            pltpu.VMEM((4, S // 2, 128), u32),
            pltpu.VMEM((NQT, D // 2, TQ), u32),
            pltpu.VMEM((NQT, D // 2, TQ), u32),
            pltpu.VMEM((NQT, D, TQ), f32),
            pltpu.VMEM((8, TQ), f32),
            pltpu.VMEM((8, 128), u32),
            pltpu.VMEM((2, TQ, D), bf16),
            pltpu.VMEM((4, 8 * len(VCH), 128), u32),
            pltpu.VMEM((DH, 8, TQ), f32),
            pltpu.VMEM((DH, 8, TQ), f32),
            pltpu.VMEM((NQT, TQ // 2, D), u32),
            pltpu.SemaphoreType.DMA((NQT,)),
            pltpu.SemaphoreType.DMA((7,)),
            pltpu.SemaphoreType.DMA((2 * NSUB,)),
        ],
        compiler_params=pltpu.CompilerParams(vmem_limit_bytes=100 * 1024 * 1024),
    )(x, A_wqkv, A_wo, B_w_gate, B_w_up, B_w_down)
    return out.reshape(1, S, D)
```

```python
import math

import jax
import jax.numpy as jnp
import jax.experimental.pallas as pl
import jax.experimental.pallas.tpu as pltpu

S, D, H, DH, F = 2048, 512, 32, 16, 1792
EPS = 1e-5
TQ = 512
NQT = S // TQ
CK = 128
NC = S // CK
NU = H * NQT
FC = 256
OFF = 2
NSUB = 2
KS = 256
QVU = 2
VCH = list(range(2, NC))
AD, ADV, AE, NG, QC, QN = 13, 12, 4, 7, 4, 8
L_LO = 2.0 ** -30
L_HI = 2.0 ** 60
F_MAX = 3.0e38
QSCALE = (DH ** -0.5) * math.log2(math.e)

f32 = jnp.float32
bf16 = jnp.bfloat16
u32 = jnp.uint32


def _ln(xf):
    m = jnp.mean(xf, axis=-1, keepdims=True)
    xc = xf - m
    v = jnp.mean(xc * xc, axis=-1, keepdims=True)
    return xc * jax.lax.rsqrt(v + EPS)


def _kernel(x_hbm, wqkv_hbm, wo_hbm, wg_hbm, wu_hbm, wd_hbm, out_hbm,
            x_v, wqkv_v, wo_v, wg_v, wu_v, wd_v, wqvt_v,
            k_v, qt_v, vt_v, ot_v, bad_v, z_v, out_v, ks_v, qb0_v, qb1_v, xn_v,
            xsem, wsem, osem):
    def x_copy(t):
        return pltpu.make_async_copy(x_hbm.at[pl.ds(t * TQ, TQ)], x_v.at[pl.ds(t * TQ, TQ)], xsem.at[t])

    def wpart_copy(j):
        return pltpu.make_async_copy(wqkv_hbm.at[:, pl.ds(j * D, D)], wqkv_v.at[j], wsem.at[j])

    w_copies = [
        pltpu.make_async_copy(wo_hbm, wo_v, wsem.at[3]),
        pltpu.make_async_copy(wg_hbm, wg_v, wsem.at[4]),
        pltpu.make_async_copy(wu_hbm, wu_v, wsem.at[5]),
        pltpu.make_async_copy(wd_hbm, wd_v, wsem.at[6]),
    ]
    x_copy(0).start()
    wpart_copy(1).start()

    z_v[...] = jnp.zeros_like(z_v)
    bad_v[...] = jnp.zeros_like(bad_v)

    def relayout_k(t):
        r0 = pl.multiple_of(t * (TQ // 2), TQ // 2)
        for g in range(4):
            kg = k_v[g * 8, pl.ds(r0, TQ // 2), :]
            for jj in range(1, 8):
                k_v[g * 8 + jj, pl.ds(r0, TQ // 2), :] = pltpu.roll(kg, 128 - DH * jj, 1)

    def ln1(t):
        xn = _ln(x_v[t * TQ:(t + 1) * TQ, :].astype(f32)).astype(bf16)
        xn_v[t] = pltpu.bitcast(xn, u32)
        return xn

    def proj_k(t, xn, lo=0, hi=TQ):
        kt = jnp.dot(xn[lo:hi], wqkv_v[1], preferred_element_type=f32).astype(bf16)
        r0, r1 = (t * TQ + lo) // 2, (t * TQ + hi) // 2
        for g in range(4):
            k_v[g * 8, r0:r1, :] = pltpu.bitcast(kt[:, g * 128:(g + 1) * 128], u32)
        for ci, c in enumerate(VCH):
            k0 = c * CK - (t * TQ + lo)
            if 0 <= k0 < hi - lo:
                kb = pltpu.bitcast(kt[k0:k0 + 16].astype(f32), u32)
                kw = (kb[0:8] >> 16) | kb[8:16]
                for g in range(4):
                    ks_v[g, ci * 8:(ci + 1) * 8, :] = kw[:, g * 128:(g + 1) * 128]

    def proj_qv(t, xn):
        qv = jax.lax.dot_general(wqvt_v[...], xn, (((1,), (1,)), ((), ())),
                                 preferred_element_type=f32)
        qt_v[t] = pltpu.bitcast((qv[0:D] * QSCALE).astype(bf16), u32)
        vt_v[t] = pltpu.bitcast(qv[D:2 * D].astype(bf16), u32)

    x_copy(0).wait()
    x_copy(1).start()
    xn0 = ln1(0)
    wpart_copy(1).wait()
    x_copy(2).start()
    proj_k(0, xn0, 0, KS)
    x_copy(1).wait()
    wpart_copy(0).start()
    wpart_copy(2).start()
    x_copy(3).start()
    xn1 = ln1(1)
    proj_k(0, xn0, KS, TQ)
    x_copy(2).wait()
    xn2 = ln1(2)
    proj_k(1, xn1)
    wpart_copy(0).wait()
    wpart_copy(2).wait()
    x_copy(3).wait()
    wqvt_v[0:D, :] = wqkv_v[0].astype(f32).T.astype(bf16)
    wqvt_v[D:2 * D, :] = wqkv_v[2].astype(f32).T.astype(bf16)
    proj_k(2, xn2)
    xn3 = ln1(3)
    proj_k(3, xn3)

    def qv_body(t, carry):
        for tt in range(QVU):
            relayout_k(t * QVU + tt)
            proj_qv(t * QVU + tt, pltpu.bitcast(xn_v[t * QVU + tt], bf16))
        return carry

    jax.lax.fori_loop(0, NQT // QVU, qv_body, 0)

    def q_rows(g, j, qt):
        return qt_v[qt, pl.ds(pl.multiple_of(g * 32 + j * 8, 8), 8), :]

    def v_chunk(h, c):
        c0 = (c * CK) % TQ
        return vt_v[(c * CK) // TQ, pl.ds(pl.multiple_of(h * 8, 8), 8), c0:c0 + CK]

    def fold(x):
        xb = pltpu.bitcast(x, u32)
        return xb[:, 0:128] | xb[:, 128:256] | xb[:, 256:384] | xb[:, 384:512]

    qbs = [qb0_v, qb1_v]

    def qb_make(g, j, qt, dst, ds, gate):
        qu = q_rows(g, j, qt)
        if gate is not None:
            qu = qu | jnp.concatenate([gate] * 4, axis=1)
        for d2 in ds:
            w = jnp.broadcast_to(qu[d2:d2 + 1, :], (8, TQ))
            dst[2 * d2] = pltpu.bitcast(w << 16, f32)
            dst[2 * d2 + 1] = pltpu.bitcast(w & jnp.uint32(0xFFFF0000), f32)

    def vchunk(g, base, qb, ci, gates):
        src = ks_v[g // 2, ci * 8:(ci + 1) * 8, :]
        base = base[g % 2]
        accs = [None, None]
        gb = None
        for d in range(DH):
            k = d * len(gates) // DH
            if gb is None or k != gb[0]:
                gb = (k, base | pltpu.bitcast(gates[k], jnp.int32))
            idx = gb[1] + d if d else gb[1]
            q = qb[d]
            w = jnp.take_along_axis(src, idx, axis=1, mode="promise_in_bounds")
            kbs = [pltpu.bitcast(w << 16, f32), pltpu.bitcast(w & jnp.uint32(0xFFFF0000), f32)]
            for r in range(2):
                t = jnp.concatenate([kbs[r]] * 4, axis=1) * q
                accs[r] = t if accs[r] is None else accs[r] + t
        return accs

    def stream(i):
        z = z_v[...]
        n_total = 8 * NC
        j = i // 4
        qt = i % 4
        base = [jnp.full((8, 128), j * DH, jnp.int32), jnp.full((8, 128), j * DH + 64, jnp.int32)]
        Gs = [(7 if (n % NC) in VCH else 8) for n in range(n_total)]
        start = [0]
        for n in range(n_total):
            start.append(start[-1] + Gs[n] + 1)
        qk_slots = set()
        for n in range(n_total):
            for gg in range(Gs[n]):
                qk_slots.add(start[n] + gg)
        deps = {}

        def add_dep(sl, v):
            while sl not in qk_slots and sl < start[-1]:
                sl += 1
            deps.setdefault(sl, []).append(v)

        pend = []
        raw = []
        sv_all = {}
        bad = None
        extra = None
        for n in range(n_total + OFF):
            if n < n_total:
                u, c = n // NC, n % NC
                g = u
                G = Gs[n]
                nv = CK - 16 * G
                if c == 0:
                    qm = pltpu.bitcast(q_rows(g, j, qt), bf16)
                    lm = None
                if QC <= c < QC + QN:
                    un = u + 1
                    if un < 8:
                        nxt = (un, j, qt)
                    else:
                        nxt = (0, jnp.minimum((i + 1) // 4, 3), (i + 1) % 4)
                    gate = pltpu.bitcast(raw[n - 2][-1], u32) & z
                    qb_make(*nxt, qbs[un % 2],
                            list(range((c - QC) * 8 // QN, (c - QC + 1) * 8 // QN)), gate)
                if c in VCH:
                    gsrc = raw[n - 1]
                    gates = [pltpu.bitcast(gsrc[(k + 1) * len(gsrc) // NG - 1], u32) & z
                             for k in range(NG)]
                    sv_all[n] = vchunk(g, base, qbs[u % 2], VCH.index(c), gates)
                rows = []
                for gg in range(G):
                    r0 = c * (CK // 2) + nv // 2 + gg * 8
                    kv = k_v[4 * g + j, r0:r0 + 8, :]
                    dl = deps.pop(start[n] + gg, [])
                    if dl:
                        dep = dl[0]
                        for x in dl[1:]:
                            dep = dep | x
                        kv = kv | (dep & z)
                    rows.append(kv)
                kc = pltpu.bitcast(jnp.concatenate(rows, axis=0), bf16)[:, 0:DH]
                s = jnp.dot(kc, qm, preferred_element_type=f32).reshape(2 * G, 8, TQ)
                raw.append([s[2 * gg + 1][:, 0:128] for gg in range(G)])
                p = jnp.exp2(s)
                if extra is not None:
                    lm = lm + extra
                    extra = None
                for gg in range(G):
                    t = p[2 * gg] + p[2 * gg + 1]
                    lm = t if lm is None else lm + t
                    if (G - 1 - gg) % AE == 0:
                        add_dep(start[n] + gg + (ADV if c in VCH else AD), fold(lm))
                pend.append((p, lm))
            m = n - OFF
            if m >= 0:
                u, c = m // NC, m % NC
                h = u * 4 + j
                if c == 0:
                    lacc = None
                    prev = None
                p, lm_m = pend[m]
                pend[m] = None
                if c in VCH:
                    pv = jnp.exp2(jnp.stack(sv_all.pop(m), axis=0))
                    lc = pv[0] + pv[1]
                    if n + 1 < n_total and (n + 1) // NC == u:
                        extra = lc
                    else:
                        lacc = lc if lacc is None else lacc + lc
                    p = jnp.concatenate([pv, p], axis=0)
                pb = p.reshape(CK, TQ).astype(bf16)
                vu = v_chunk(h, c)
                if prev is not None:
                    vu = vu | (fold(prev) & z)
                prev = lacc if (c in VCH and extra is None) else None
                r = jnp.dot(pltpu.bitcast(vu, bf16), pb, preferred_element_type=f32)
                acc = r if c == 0 else acc + r
                if c == NC - 1:
                    lf = lm_m if lacc is None else lm_m + lacc
                    l = jnp.sum(lf, axis=0, keepdims=True)
                    o = acc * (1.0 / l)
                    ot_v[qt, pl.ds(pl.multiple_of(h * DH, DH), DH), :] = o
                    ok_l = jnp.logical_and(l >= L_LO, l <= L_HI)
                    ok_o = jnp.abs(o) <= F_MAX
                    b = (jnp.where(ok_o[0:8], 0.0, 1.0) + jnp.where(ok_o[8:16], 0.0, 1.0)
                         + jnp.where(ok_l, 0.0, 1.0))
                    bad = b if bad is None else bad + b
        bad_v[...] = bad_v[...] + bad

    qb_make(0, 0, 0, qb0_v, range(8), None)

    def attn_body(i, carry):
        @pl.when(i == 1)
        def _():
            for c in w_copies:
                c.start()

        stream(i)
        return carry

    jax.lax.fori_loop(0, 16, attn_body, 0)

    @pl.when(jnp.max(bad_v[...]) > 0.0)
    def _():
        def safe_unit(u, carry):
            h, qt = u // NQT, u % NQT
            qm = pltpu.bitcast(q_rows(h // 4, h % 4, qt), bf16)
            kg = pltpu.bitcast(k_v[h], bf16)[:, 0:DH]
            s = jnp.dot(kg, qm, preferred_element_type=f32)
            p = jnp.exp2(s - jnp.max(s, axis=0, keepdims=True))
            l = jnp.sum(p, axis=0, keepdims=True)
            pb = p.astype(bf16)
            acc = None
            for t in range(NQT):
                vv = pltpu.bitcast(vt_v[t, pl.ds(pl.multiple_of(h * 8, 8), 8), :], bf16)
                r = jnp.dot(vv, pb[t * TQ:(t + 1) * TQ], preferred_element_type=f32)
                acc = r if acc is None else acc + r
            ot_v[qt, pl.ds(pl.multiple_of(h * DH, DH), DH), :] = acc / l
            return carry

        jax.lax.fori_loop(0, NU, safe_unit, 0)

    for c in w_copies:
        c.wait()

    HR = TQ // NSUB

    def out_copy(t, a):
        return pltpu.make_async_copy(out_v.at[t % 2, pl.ds(a * HR, HR)],
                                     out_hbm.at[pl.ds(t * TQ + a * HR, HR)], osem.at[(t % 2) * NSUB + a])

    def phase_c(t, carry):
        r0 = pl.multiple_of(t * TQ, TQ)

        @pl.when(t >= 2)
        def _():
            for a in range(NSUB):
                out_copy(t - 2, a).wait()

        hres = []
        for a in range(NSUB):
            o = ot_v[t, :, a * HR:(a + 1) * HR].T.astype(bf16)
            attn = jnp.dot(o, wo_v[...], preferred_element_type=f32)
            hres.append(x_v[pl.ds(r0 + a * HR, HR), :].astype(f32) + attn)
        ys = []
        for a in range(NSUB):
            hn = _ln(hres[a]).astype(bf16)
            y = hres[a]
            for fc in range(F // FC):
                gate = jnp.dot(hn, wg_v[:, fc * FC:(fc + 1) * FC], preferred_element_type=f32)
                up = jnp.dot(hn, wu_v[:, fc * FC:(fc + 1) * FC], preferred_element_type=f32)
                hg = 0.5 * gate
                act = ((hg + hg * jnp.tanh(hg)) * up).astype(bf16)
                y = y + jnp.dot(act, wd_v[fc * FC:(fc + 1) * FC, :], preferred_element_type=f32)
            ys.append(y.astype(bf16))
        for a in range(NSUB):
            out_v[t % 2, a * HR:(a + 1) * HR, :] = ys[a]
            out_copy(t, a).start()
        return carry

    jax.lax.fori_loop(0, NQT, phase_c, 0)
    for t in range(NQT - 2, NQT):
        for a in range(NSUB):
            out_copy(t, a).wait()


@jax.jit
def pallas_sequential_preLN__softmax_full_mha__swiglu_ffn__prompt_kernel(
    A_x: jax.Array,
    A_wqkv: jax.Array,
    A_wo: jax.Array,
    B_x: jax.Array,
    B_w_gate: jax.Array,
    B_w_up: jax.Array,
    B_w_down: jax.Array,
):
    del B_x
    x = A_x.reshape(S, D)
    any_spec = pl.BlockSpec(memory_space=pl.ANY)
    out = pl.pallas_call(
        _kernel,
        out_shape=jax.ShapeDtypeStruct((S, D), bf16),
        in_specs=[any_spec] * 6,
        out_specs=any_spec,
        scratch_shapes=[
            pltpu.VMEM((S, D), bf16),
            pltpu.VMEM((3, D, D), bf16),
            pltpu.VMEM((D, D), bf16),
            pltpu.VMEM((D, F), bf16),
            pltpu.VMEM((D, F), bf16),
            pltpu.VMEM((F, D), bf16),
            pltpu.VMEM((2 * D, D), bf16),
            pltpu.VMEM((H, S // 2, 128), u32),
            pltpu.VMEM((NQT, D // 2, TQ), u32),
            pltpu.VMEM((NQT, D // 2, TQ), u32),
            pltpu.VMEM((NQT, D, TQ), f32),
            pltpu.VMEM((8, TQ), f32),
            pltpu.VMEM((8, 128), u32),
            pltpu.VMEM((2, TQ, D), bf16),
            pltpu.VMEM((4, 8 * len(VCH), 128), u32),
            pltpu.VMEM((DH, 8, TQ), f32),
            pltpu.VMEM((DH, 8, TQ), f32),
            pltpu.VMEM((NQT, TQ // 2, D), u32),
            pltpu.SemaphoreType.DMA((NQT,)),
            pltpu.SemaphoreType.DMA((7,)),
            pltpu.SemaphoreType.DMA((2 * NSUB,)),
        ],
        compiler_params=pltpu.CompilerParams(vmem_limit_bytes=100 * 1024 * 1024),
    )(x, A_wqkv, A_wo, B_w_gate, B_w_up, B_w_down)
    return out.reshape(1, S, D)
```
